```python
import os as _os
_os.environ.setdefault("JAX_PLATFORMS", "cpu")
import jax
import jax.numpy as jnp

def _softmax(x, axis=-1):
    return jax.nn.softmax(x, axis=axis)
def _gelu(x):
    return jax.nn.gelu(x, approximate=True)
def _silu(x):
    return jax.nn.silu(x)
def _sigmoid(x):
    return jax.nn.sigmoid(x)
def _layernorm(x, axis=-1, eps=1e-5):
    m = jnp.mean(x, axis=axis, keepdims=True)
    v = jnp.var(x, axis=axis, keepdims=True)
    return (x - m) / jnp.sqrt(v + eps)
def _scatter_add(tgt, idx, src, axis=0):
    return tgt.at[idx].add(src)
def _segment_sum(src, seg, n):
    return jax.ops.segment_sum(src, seg, n)
class _Rng:
    def __init__(self, key):
        self._k = key
    def _next(self):
        self._k, sub = jax.random.split(self._k)
        return sub
    def normal(self, shape):
        return jax.random.normal(self._next(), shape, dtype=jnp.bfloat16)
    def randint(self, lo, hi, shape):
        return jax.random.randint(self._next(), shape, lo, hi, dtype=jnp.int32)
    def uniform(self, shape, lo=0.0, hi=1.0):
        return jax.random.uniform(self._next(), shape, jnp.bfloat16, lo, hi)
    def permutation(self, n):
        return jax.random.permutation(self._next(), n)


kernel_name = 'standalone__dense_activation_silu__prompt'

def setup_inputs():
    _rng = _Rng(jax.random.key(int.from_bytes(__import__("os").urandom(4), "little")))
    _w = (lambda a: (lambda t: t.astype(jnp.bfloat16) if jnp.issubdtype(t.dtype, jnp.floating) else t)(jnp.asarray(a)))
    B, S, D, F = 1, 2048, 448, 1792
    return {
        "x": _w((lambda *s: _rng.normal(s) * 0.05)(B, S, D)),
        "w1": _w((lambda *s: _rng.normal(s) * 0.05)(D, F) * (D ** -0.5)),
        "w2": _w((lambda *s: _rng.normal(s) * 0.05)(F, D) * (F ** -0.5)),
    }

def reference(x, w1, w2):
    h = jnp.einsum("bsd,df->bsf", x, w1)
    h = _silu(h)
    out = jnp.einsum("bsf,fd->bsd", h, w2)
    return out
```

```python
import contextlib
import jax, jax.numpy as jnp
from jax.experimental import pallas as pl
from jax.experimental.pallas import tpu as pltpu
D, S, F = 448, 2048, 1792
DP = 512; KH = 256; FH = F // 2; DH = D // 2
bf = jnp.bfloat16; f32 = jnp.float32

def act(h):
    hh = 0.5 * h
    return hh + hh * jnp.tanh(hh)

def dot(a, b):
    return jnp.dot(a, b, preferred_element_type=f32)

def add(u, v): return (u.astype(f32) + v.astype(f32)).astype(bf)
def sub(u, v): return (u.astype(f32) - v.astype(f32)).astype(bf)
def cat(xs, axis): return xs[0] if len(xs) == 1 else jnp.concatenate(xs, axis=axis)

def make(stages=((256, 128), (512, 256), (1024, 512)), tiles=(256, 256, 512, 512, 512), scopes=False, xpad=128):
    assert sum(tiles) == S
    tstart = [sum(tiles[:i]) for i in range(len(tiles))]
    nst = len(stages)
    all_stages = list(stages) + [(S, FH)]
    for (s_end, g_end) in all_stages:
        assert s_end in tstart + [S]
    ntile = len(tiles)
    scope = (lambda n: jax.named_scope(n)) if scopes else (lambda n: contextlib.nullcontext())

    def kernel(xt_hbm, w1_hbm, w2t_hbm, o_hbm, xt_v, w1_v, w2t_v, o_v, sems):
        def in_copies(k):
            s0, g0 = (0, 0) if k == 0 else all_stages[k - 1]
            s1, g1 = all_stages[k]
            cps = []
            if g1 > g0:
                cps.append(pltpu.make_async_copy(w1_hbm.at[:, pl.ds(g0, g1 - g0)], w1_v.at[pl.ds(0, D), pl.ds(g0, g1 - g0)], sems.at[k]))
                cps.append(pltpu.make_async_copy(w1_hbm.at[:, pl.ds(FH + g0, g1 - g0)], w1_v.at[pl.ds(0, D), pl.ds(FH + g0, g1 - g0)], sems.at[k]))
            if s1 > s0:
                cps.append(pltpu.make_async_copy(xt_hbm.at[:, pl.ds(s0, s1 - s0)], xt_v.at[pl.ds(0, D), pl.ds(s0, s1 - s0)], sems.at[k]))
            if k == nst:
                cps.append(pltpu.make_async_copy(w2t_hbm, w2t_v, sems.at[k]))
            return cps
        def out_copy(j, q):
            s0, w = tstart[j], tiles[j] // 2
            r0 = (q // 2) * DH; c0 = s0 + (q % 2) * w
            return pltpu.make_async_copy(o_v.at[pl.ds(r0, DH), pl.ds(c0, w)], o_hbm.at[pl.ds(r0, DH), pl.ds(c0, w)], sems.at[0])

        for k in range(nst + 1):
            for c in in_copies(k):
                c.start()
        xt_v[D:DP, :S] = jnp.zeros((DP - D, S), bf)
        w1_v[D:DP, :] = jnp.zeros((DP - D, F), bf)

        A1 = []
        B1 = {}
        H = {j: [] for j in range(ntile)}

        def prep_w1(g0, g1):
            top = w1_v[:, g0:g1].T
            bot = w1_v[:, FH + g0:FH + g1].T
            a11, a12 = top[:, :KH], top[:, KH:]
            a21, a22 = bot[:, :KH], bot[:, KH:]
            A1.append((g0, g1, [add(a11, a22), add(a21, a22), a11, a22, add(a11, a12), sub(a21, a11), sub(a12, a22)]))

        def prep_x(j):
            s0, w = tstart[j], tiles[j] // 2
            b11 = xt_v[:KH, s0:s0 + w]; b12 = xt_v[:KH, s0 + w:s0 + 2 * w]
            b21 = xt_v[KH:, s0:s0 + w]; b22 = xt_v[KH:, s0 + w:s0 + 2 * w]
            B1[j] = [add(b11, b22), b11, sub(b12, b22), sub(b21, b11), b22, add(b11, b12), add(b21, b22)]

        def mm1(g0, g1, j):
            parts = [a for (a0, a1, a) in A1 if g0 <= a0 and a1 <= g1]
            A = [cat([p[i] for p in parts], 0) for i in range(7)]
            Bs = B1[j]
            m1 = dot(A[0], Bs[0])
            m4 = dot(A[3], Bs[3])
            m5 = dot(A[4], Bs[4])
            m7 = dot(A[6], Bs[6])
            h11 = act(m1 + m4 - m5 + m7)
            m3 = dot(A[2], Bs[2])
            h12 = act(m3 + m5)
            m2 = dot(A[1], Bs[1])
            h21 = act(m2 + m4)
            m6 = dot(A[5], Bs[5])
            h22 = act(m1 - m2 + m3 + m6)
            H[j].append((g0, g1, [(h11 + h22).astype(bf), h11.astype(bf), (h12 - h22).astype(bf), (h21 - h11).astype(bf),
                                  h22.astype(bf), (h11 + h12).astype(bf), (h21 + h22).astype(bf)]))

        A2 = []
        def prep_w2():
            a11 = w2t_v[:DH, :FH]; a12 = w2t_v[:DH, FH:]
            a21 = w2t_v[DH:, :FH]; a22 = w2t_v[DH:, FH:]
            A2.extend([add(a11, a22), add(a21, a22), a11, a22, add(a11, a12), sub(a21, a11), sub(a12, a22)])

        def mm2(j):
            s0, w = tstart[j], tiles[j] // 2
            parts = sorted(H[j], key=lambda t: t[0])
            Hs = [cat([p[2][i] for p in parts], 0) for i in range(7)]
            m2 = dot(A2[1], Hs[1])
            m4 = dot(A2[3], Hs[3])
            o_v[DH:, s0:s0 + w] = (m2 + m4).astype(bf)
            out_copy(j, 2).start()
            m6 = dot(A2[5], Hs[5])
            m1 = dot(A2[0], Hs[0])
            m3 = dot(A2[2], Hs[2])
            o_v[DH:, s0 + w:s0 + 2 * w] = (m1 - m2 + m3 + m6).astype(bf)
            out_copy(j, 3).start()
            m5 = dot(A2[4], Hs[4])
            o_v[:DH, s0 + w:s0 + 2 * w] = (m3 + m5).astype(bf)
            out_copy(j, 1).start()
            m7 = dot(A2[6], Hs[6])
            o_v[:DH, s0:s0 + w] = (m1 + m4 - m5 + m7).astype(bf)
            out_copy(j, 0).start()

        for k in range(nst + 1):
          with scope(f"wait{k}"):
            for c in in_copies(k):
                c.wait()
          with scope(f"stage{k}"):
            s0, g0 = (0, 0) if k == 0 else all_stages[k - 1]
            s1, g1 = all_stages[k]
            old_tiles = [j for j in range(ntile) if tstart[j] < s0]
            new_tiles = [j for j in range(ntile) if s0 <= tstart[j] < s1]
            if k < nst:
                for j in new_tiles: prep_x(j)
                if g0 > 0:
                    for j in new_tiles: mm1(0, g0, j)
                if g1 > g0:
                    prep_w1(g0, g1)
                    for j in old_tiles + new_tiles: mm1(g0, g1, j)
            else:
                first_new = new_tiles[0]
                prep_x(first_new)
                mm1(0, g0, first_new)
                prep_w1(g0, g1)
                prep_w2()
                for j in range(ntile):
                    if j in new_tiles and j != first_new:
                        prep_x(j)
                        mm1(0, g1, j)
                    else:
                        mm1(g0, g1, j)
                    mm2(j)
        with scope("waitout"):
            pltpu.make_async_copy(o_v, o_hbm, sems.at[0]).wait()

    def fn(x, w1, w2):
        B = x.shape[0]
        xt = x.reshape(S, D).T
        w2t = w2.T
        out = pl.pallas_call(kernel,
            in_specs=[pl.BlockSpec(memory_space=pl.ANY)]*3,
            out_specs=pl.BlockSpec(memory_space=pl.ANY),
            out_shape=jax.ShapeDtypeStruct((D, S), x.dtype),
            scratch_shapes=[pltpu.VMEM((DP, S + xpad), bf), pltpu.VMEM((DP, F), bf), pltpu.VMEM((D, F), bf), pltpu.VMEM((D, S), bf),
                            pltpu.SemaphoreType.DMA((nst + 1,))],
            compiler_params=pltpu.CompilerParams(vmem_limit_bytes=120*1024*1024),
        )(xt, w1, w2t)
        return out.T.reshape(B, S, D)
    return fn


_impl = make()


@jax.jit
def pallas_standalone__dense_activation_silu__prompt_kernel(x, w1, w2):
    return _impl(x, w1, w2)
```

```python
import contextlib
import jax, jax.numpy as jnp
from jax.experimental import pallas as pl
from jax.experimental.pallas import tpu as pltpu
D, S, F = 448, 2048, 1792
DP = 512; KH = 256; FH = F // 2; DH = D // 2
bf = jnp.bfloat16; f32 = jnp.float32

def dot(a, b): return jnp.dot(a, b, preferred_element_type=f32)
def add(u, v): return (u.astype(f32) + v.astype(f32)).astype(bf)
def sub(u, v): return (u.astype(f32) - v.astype(f32)).astype(bf)

ORD = dict(std=(0, 3, 4, 6, 2, 1, 5),
           nb=(1, 4, 3, 0, 6, 2, 5),
           na=(2, 3, 4, 0, 6, 1, 5))

def make(tiles, plan, scopes=False, xpad=128, half=False, order2=(1, 3, 5, 0, 2, 4, 6), outq=True, hscr=True, hpad=128, asplit=True):
    assert sum(tiles) == S
    tstart = [sum(tiles[:i]) for i in range(len(tiles) + 1)]
    nst = len(plan)
    scope = (lambda n: jax.named_scope(n)) if scopes else (lambda n: contextlib.nullcontext())
    def act(h):
        hh = h if half else 0.5 * h
        return hh + hh * jnp.tanh(hh)

    def kernel(xt_hbm, w1_hbm, w2t_hbm, o_hbm, xt_v, w1_v, w2t_v, o_v, hs_v, sems):
        def in_copies(k):
            cps = []
            for ld in plan[k][0]:
                if ld[0] in ('w1', 'w2'):
                    src, dst = (w1_hbm, w1_v) if ld[0] == 'w1' else (w2t_hbm, w2t_v)
                    g0, g1 = ld[1:]
                    if g0 == 0 and g1 == FH:
                        cps.append(pltpu.make_async_copy(src, dst.at[pl.ds(0, D), :], sems.at[k]))
                    else:
                        for off in (0, FH):
                            cps.append(pltpu.make_async_copy(src.at[:, pl.ds(off + g0, g1 - g0)], dst.at[pl.ds(0, D), pl.ds(off + g0, g1 - g0)], sems.at[k]))
                elif ld[0] == 'x':
                    s0, s1 = tstart[ld[1]], tstart[ld[2]]
                    cps.append(pltpu.make_async_copy(xt_hbm.at[:, pl.ds(s0, s1 - s0)], xt_v.at[pl.ds(0, D), pl.ds(s0, s1 - s0)], sems.at[k]))
            return cps
        def out_copy(r0, nr, c0, w):
            return pltpu.make_async_copy(o_v.at[pl.ds(r0, nr), pl.ds(c0, w)], o_hbm.at[pl.ds(r0, nr), pl.ds(c0, w)], sems.at[0])

        for k in range(nst):
            for c in in_copies(k):
                c.start()
        xt_v[D:DP, :S] = jnp.zeros((DP - D, S), bf)
        w1_v[D:DP, :] = jnp.zeros((DP - D, F), bf)

        A1 = []; A2 = []; B1 = {}; H = {}; ACC = {}; KDONE = {}; DEFER = []

        def gather(lst, g0, g1, i, axis):
            parts = []
            for (a0, a1, arrs) in sorted(lst, key=lambda t: t[0]):
                lo, hi = max(a0, g0), min(a1, g1)
                if lo < hi:
                    v = arrs[i]
                    if (lo, hi) != (a0, a1):
                        v = v[lo - a0:hi - a0] if axis == 0 else v[:, lo - a0:hi - a0]
                    parts.append(v)
            assert sum(p.shape[axis] for p in parts) == g1 - g0
            return parts[0] if len(parts) == 1 else jnp.concatenate(parts, axis=axis)

        def pw1(g0, g1):
            top = w1_v[:, g0:g1].T
            bot = w1_v[:, FH + g0:FH + g1].T
            if half:
                top = top.astype(f32) * 0.5; bot = bot.astype(f32) * 0.5
            a11, a12 = top[:, :KH], top[:, KH:]
            a21, a22 = bot[:, :KH], bot[:, KH:]
            A1.append((g0, g1, [add(a11, a22), add(a21, a22), a11.astype(bf), a22.astype(bf), add(a11, a12), sub(a21, a11), sub(a12, a22)]))

        def pw2(g0, g1):
            a11 = w2t_v[:DH, g0:g1]; a12 = w2t_v[:DH, FH + g0:FH + g1]
            a21 = w2t_v[DH:, g0:g1]; a22 = w2t_v[DH:, FH + g0:FH + g1]
            A2.append((g0, g1, [add(a11, a22), add(a21, a22), a11, a22, add(a11, a12), sub(a21, a11), sub(a12, a22)]))

        def px(j):
            s0, w = tstart[j], tiles[j] // 2
            b11 = xt_v[:KH, s0:s0 + w]; b12 = xt_v[:KH, s0 + w:s0 + 2 * w]
            b21 = xt_v[KH:, s0:s0 + w]; b22 = xt_v[KH:, s0 + w:s0 + 2 * w]
            B1[j] = [add(b11, b22), b11, sub(b12, b22), sub(b21, b11), b22, add(b11, b12), add(b21, b22)]

        def puth(j, g0, g1, h11, h12, h21, h22):
            vals = [(h11 + h22).astype(bf), h11.astype(bf), (h12 - h22).astype(bf), (h21 - h11).astype(bf),
                    h22.astype(bf), (h11 + h12).astype(bf), (h21 + h22).astype(bf)]
            if hscr:
                c0, w = tstart[j] // 2, tiles[j] // 2
                for i in (1, 5, 3, 0, 2, 4, 6):
                    hs_v[i, g0:g1, c0:c0 + w] = vals[i]
            else:
                H.setdefault(j, []).append((g0, g1, vals))

        def geth(j, g0, g1, i):
            if hscr:
                c0, w = tstart[j] // 2, tiles[j] // 2
                return hs_v[i, g0:g1, c0:c0 + w]
            return gather(H[j], g0, g1, i, 0)

        def mm1(g0, g1, j, order='std', defer=False):
            if asplit:
                chunks = [(max(a0, g0), min(a1, g1)) for (a0, a1, _) in sorted(A1, key=lambda t: t[0]) if max(a0, g0) < min(a1, g1)]
                if len(chunks) > 1:
                    for n, (c0, c1) in enumerate(chunks):
                        mm1(c0, c1, j, order if n == 0 else 'std', defer and n == len(chunks) - 1)
                    return
            order = ORD[order]
            m = [None] * 7
            h = {}
            need = {'11': (0, 3, 4, 6), '12': (2, 4), '21': (1, 3), '22': (0, 1, 2, 5)}
            def comb(q):
                m1, m2, m3, m4, m5, m6, m7 = m
                return {'11': lambda: m1 + m4 - m5 + m7, '12': lambda: m3 + m5, '21': lambda: m2 + m4, '22': lambda: m1 - m2 + m3 + m6}[q]()
            for n, i in enumerate(order):
                m[i] = dot(gather(A1, g0, g1, i, 0), B1[j][i])
                if n == 6 and defer: break
                for q, nd in need.items():
                    if q not in h and all(m[t] is not None for t in nd):
                        h[q] = act(comb(q))
            def finish():
                for q in need:
                    if q not in h: h[q] = act(comb(q))
                h11, h12, h21, h22 = h['11'], h['12'], h['21'], h['22']
                puth(j, g0, g1, h11, h12, h21, h22)
            if defer: DEFER.append(finish)
            else: finish()

        def mm1m(g0, g1, js, order='std'):
            order = ORD[order]
            ms = {j: [None] * 7 for j in js}
            for i in order:
                a = gather(A1, g0, g1, i, 0)
                for j in js:
                    ms[j][i] = dot(a, B1[j][i])
            for j in js:
                m1, m2, m3, m4, m5, m6, m7 = ms[j]
                h11 = act(m1 + m4 - m5 + m7); h12 = act(m3 + m5); h21 = act(m2 + m4); h22 = act(m1 - m2 + m3 + m6)
                puth(j, g0, g1, h11, h12, h21, h22)

        def flush():
            while DEFER: DEFER.pop(0)()

        def mm2(g0, g1, j, order=None):
            order = order or order2
            s0, w = tstart[j], tiles[j] // 2
            acc = ACC.setdefault(j, [None] * 7)
            KDONE[j] = KDONE.get(j, 0) + g1 - g0
            last = KDONE[j] == FH
            for n, i in enumerate(order):
                p = dot(gather(A2, g0, g1, i, 1), geth(j, g0, g1, i))
                acc[i] = p if acc[i] is None else acc[i] + p
                if last:
                    m1, m2, m3, m4, m5, m6, m7 = acc
                    done = set(order[:n + 1])
                    fin = lambda need: i in need and set(need) <= done
                    for need, r0, c0, val in (((1, 3), DH, s0, lambda: m2 + m4),
                                              ((0, 1, 2, 5), DH, s0 + w, lambda: m1 - m2 + m3 + m6),
                                              ((2, 4), 0, s0 + w, lambda: m3 + m5),
                                              ((0, 3, 4, 6), 0, s0, lambda: m1 + m4 - m5 + m7)):
                        if fin(need):
                            o_v[r0:r0 + DH, c0:c0 + w] = val().astype(bf)
                            if outq: out_copy(r0, DH, c0, w).start()
            if last and not outq:
                out_copy(0, D, s0, 2 * w).start()

        fns = dict(mm1m=mm1m, px=px, pw1=pw1, pw2=pw2, mm1=mm1, mm2=mm2)
        for k in range(nst):
            with scope(f"wait{k}"):
                for c in in_copies(k):
                    c.wait()
            with scope(f"stage{k}"):
                flush()
                for op in plan[k][1]:
                    fns[op[0]](*op[1:])
        assert all(KDONE.get(j) == FH for j in range(len(tiles))), KDONE
        with scope("waitout"):
            pltpu.make_async_copy(o_v, o_hbm, sems.at[0]).wait()

    def fn(x, w1, w2):
        B = x.shape[0]
        xt = x.reshape(S, D).T
        w2t = w2.T
        out = pl.pallas_call(kernel,
            in_specs=[pl.BlockSpec(memory_space=pl.ANY)]*3,
            out_specs=pl.BlockSpec(memory_space=pl.ANY),
            out_shape=jax.ShapeDtypeStruct((D, S), x.dtype),
            scratch_shapes=[pltpu.VMEM((DP, S + xpad), bf), pltpu.VMEM((DP, F), bf), pltpu.VMEM((D, F), bf), pltpu.VMEM((D, S), bf), pltpu.VMEM((7, FH, S // 2 + hpad), bf),
                            pltpu.SemaphoreType.DMA((nst,))],
            compiler_params=pltpu.CompilerParams(vmem_limit_bytes=120*1024*1024),
        )(xt, w1, w2t)
        return out.T.reshape(B, S, D)
    return fn

T5 = (256, 256, 512, 512, 512)
def planC(v=0, df=True, **kw):
    plan = [
        ([('w1', 0, 128), ('x', 0, 1)], [('px', 0), ('pw1', 0, 128), ('mm1', 0, 128, 0, 'na', df)]),
        ([('w1', 128, 256), ('x', 1, 2)], [('px', 1), ('mm1', 0, 128, 1, 'nb'), ('pw1', 128, 256), ('mm1', 128, 256, 0, 'na'), ('mm1', 128, 256, 1, 'std', df)]),
        ([('w1', 256, 512), ('x', 2, 3)], [('px', 2), ('mm1', 0, 256, 2, 'nb'), ('pw1', 256, 512), ('mm1', 256, 512, 0, 'na'), ('mm1', 256, 512, 1), ('mm1', 256, 512, 2, 'std', df)]),
    ]
    L3 = [('w1', 512, 896), ('x', 3, 5), ('w2', 0, 896)]
    if v == 0:
        ops = [('px', 3), ('mm1', 0, 512, 3, 'nb'), ('pw1', 512, 896), ('pw2', 0, 896), ('mm1', 512, 896, 0, 'na'), ('mm2', 0, 896, 0), ('mm1', 512, 896, 1), ('mm2', 0, 896, 1),
               ('mm1', 512, 896, 2), ('mm2', 0, 896, 2), ('mm1', 512, 896, 3), ('mm2', 0, 896, 3), ('px', 4), ('mm1', 0, 896, 4), ('mm2', 0, 896, 4)]
    if v == 1:
        ops = [('px', 3), ('mm1', 0, 512, 3, 'nb'), ('pw1', 512, 896), ('pw2', 0, 896), ('mm1', 512, 896, 3, 'na'), ('mm1', 512, 896, 0), ('mm2', 0, 896, 0, (3, 2, 1, 5, 0, 4, 6)), ('mm1', 512, 896, 1), ('mm2', 0, 896, 1),
               ('mm1', 512, 896, 2), ('mm2', 0, 896, 2), ('mm2', 0, 896, 3), ('px', 4), ('mm1', 0, 896, 4), ('mm2', 0, 896, 4)]
    plan.append((L3, ops))
    return make(T5, plan, **kw)


def planD(v=0, **kw):
    L3 = [('w1', 512, 896), ('x', 3, 5), ('w2', 0, 896)]
    ops3 = [('px', 3), ('mm1', 0, 512, 3, 'nb'), ('pw1', 512, 896), ('pw2', 0, 896), ('mm1', 512, 896, 3, 'na'), ('mm1', 512, 896, 0), ('mm2', 0, 896, 0, (3, 2, 1, 5, 0, 4, 6)), ('mm1', 512, 896, 1), ('mm2', 0, 896, 1),
               ('mm1', 512, 896, 2), ('mm2', 0, 896, 2), ('mm2', 0, 896, 3), ('px', 4), ('mm1', 0, 896, 4), ('mm2', 0, 896, 4)]
    s0 = ([('w1', 0, 128), ('x', 0, 1)], [('px', 0), ('pw1', 0, 128), ('mm1', 0, 128, 0, 'na')])
    if v == 0:
        plan = [s0,
        ([('w1', 128, 256), ('x', 1, 2)], [('px', 1), ('mm1', 0, 128, 1, 'nb'), ('pw1', 128, 256), ('mm1m', 128, 256, (0, 1), 'na')]),
        ([('w1', 256, 512), ('x', 2, 3)], [('px', 2), ('mm1', 0, 256, 2, 'nb'), ('pw1', 256, 512), ('mm1m', 256, 512, (0, 1), 'na'), ('mm1', 256, 512, 2, 'std')]),
        (L3, ops3)]
    if v == 1:
        plan = [s0,
        ([('w1', 128, 256), ('x', 1, 2)], [('px', 1), ('mm1', 0, 128, 1, 'nb'), ('pw1', 128, 256), ('mm1m', 128, 256, (0, 1), 'na')]),
        ([('w1', 256, 512), ('x', 2, 3)], [('px', 2), ('mm1', 0, 256, 2, 'nb'), ('pw1', 256, 512), ('mm1', 256, 512, 2, 'na'), ('mm1m', 256, 512, (0, 1), 'std')]),
        (L3, ops3)]
    if v == 2:
        plan = [s0,
        ([('w1', 128, 256), ('x', 1, 2)], [('px', 1), ('mm1', 0, 128, 1, 'nb'), ('pw1', 128, 256), ('mm1m', 128, 256, (0, 1), 'na')]),
        ([('w1', 256, 512), ('x', 2, 3)], [('px', 2), ('mm1', 0, 256, 2, 'nb'), ('pw1', 256, 384), ('pw1', 384, 512), ('mm1', 256, 384, 2, 'na'), ('mm1m', 256, 384, (0, 1), 'std'),
                                            ('mm1', 384, 512, 2, 'na'), ('mm1m', 384, 512, (0, 1), 'std')]),
        (L3, ops3)]
    if v == 3:
        plan = [s0,
        ([('w1', 128, 256), ('x', 1, 2)], [('px', 1), ('mm1', 0, 128, 1, 'nb'), ('pw1', 128, 256), ('mm1m', 128, 256, (0, 1), 'na')]),
        ([('w1', 256, 512), ('x', 2, 3)], [('px', 2), ('mm1', 0, 256, 2, 'nb'), ('pw1', 256, 512), ('mm1m', 256, 512, (2, 0, 1), 'na')]),
        (L3, ops3)]
    return make(T5, plan, **kw)


def auto(tiles, stages, w2stage=None, final='a', o2first=(3, 2, 1, 5, 0, 4, 6), split0=False, **kw):
    nt = len(tiles)
    full = list(stages) + [(nt, FH)]
    if split0:
        full = [(0, full[0][1])] + full
    plan = []
    for k, (t1, g1) in enumerate(full):
        t0, g0 = (0, 0) if k == 0 else full[k - 1]
        loads = []
        if g1 > g0: loads.append(('w1', g0, g1))
        if t1 > t0: loads.append(('x', t0, t1))
        last = k == len(full) - 1
        if last: loads.append(('w2', 0, FH))
        ops = []
        newt = list(range(t0, t1)); oldt = list(range(0, t0))
        if not last:
            for n, j in enumerate(newt):
                ops.append(('px', j))
                if g0 > 0: ops.append(('mm1', 0, g0, j, 'nb' if n == 0 else 'std'))
            if g1 > g0:
                ops.append(('pw1', g0, g1))
                order = sorted(oldt + newt, key=lambda j: -tiles[j])
                for n, j in enumerate(order):
                    ops.append(('mm1', g0, g1, j, 'na' if n == 0 else 'std'))
        else:
            first = newt[0] if newt else None
            done1 = set()
            if first is not None:
                ops += [('px', first), ('mm1', 0, g0, first, 'nb')]
            if g1 > g0: ops.append(('pw1', g0, g1))
            ops.append(('pw2', 0, FH))
            if g1 > g0 and first is not None and final == 'a':
                ops.append(('mm1', g0, g1, first, 'na')); done1.add(first)
            n2 = 0
            for j in range(nt):
                if j not in done1:
                    if j in newt and j != first:
                        ops += [('px', j), ('mm1', 0, FH, j)]
                    elif g1 > g0:
                        ops.append(('mm1', g0, g1, j))
                ops.append(('mm2', 0, FH, j) + ((o2first,) if n2 == 0 else ()))
                n2 += 1
        plan.append((loads, ops))
    return make(tuple(tiles), plan, **kw)


_impl = auto((256,256,512,512,512),[(1,128),(2,256),(3,384),(4,896)],split0=True)


@jax.jit
def pallas_standalone__dense_activation_silu__prompt_kernel(x, w1, w2):
    return _impl(x, w1, w2)
```

```python
import contextlib
import jax, jax.numpy as jnp
from jax.experimental import pallas as pl
from jax.experimental.pallas import tpu as pltpu
D, S, F = 448, 2048, 1792
KT = 128; FH = F // 2; DH = D // 2
bf = jnp.bfloat16; f32 = jnp.float32

def dot(a, b): return jnp.dot(a, b, preferred_element_type=f32)
def add(u, v): return (u.astype(f32) + v.astype(f32)).astype(bf)
def sub(u, v): return (u.astype(f32) - v.astype(f32)).astype(bf)
def act(h):
    hh = 0.5 * h
    return hh + hh * jnp.tanh(hh)

ORD = dict(std=(0, 3, 4, 7, 6, 2, 8, 1, 5),
           nb=(7, 4, 8, 1, 3, 0, 6, 2, 5),
           na=(3, 2, 7, 4, 0, 6, 8, 1, 5))

def make(tiles, plan, scopes=False, xpad=128, order2=(1, 3, 5, 0, 2, 4, 6), hpad=128, lastsplit=(2, 128), bigfirst=True, ords=None):
    assert sum(tiles) == S
    tstart = [sum(tiles[:i]) for i in range(len(tiles) + 1)]
    nst = len(plan)
    scope = (lambda n: jax.named_scope(n)) if scopes else (lambda n: contextlib.nullcontext())
    ORDS = dict(ORD); ORDS.update(ords or {})

    def kernel(xt_hbm, w1_hbm, w2t_hbm, o_hbm, xt_v, w1_v, w2t_v, o_v, hs_v, sems):
        def in_copies(k):
            cps = []
            for ld in plan[k][0]:
                if ld[0] in ('w1', 'w2'):
                    src, dst = (w1_hbm, w1_v) if ld[0] == 'w1' else (w2t_hbm, w2t_v)
                    g0, g1 = ld[1:]
                    if g0 == 0 and g1 == FH:
                        cps.append(pltpu.make_async_copy(src, dst, sems.at[k]))
                    else:
                        for off in (0, FH):
                            cps.append(pltpu.make_async_copy(src.at[:, pl.ds(off + g0, g1 - g0)], dst.at[:, pl.ds(off + g0, g1 - g0)], sems.at[k]))
                elif ld[0] == 'x':
                    s0, s1 = tstart[ld[1]], tstart[ld[2]]
                    cps.append(pltpu.make_async_copy(xt_hbm.at[:, pl.ds(s0, s1 - s0)], xt_v.at[:, pl.ds(s0, s1 - s0)], sems.at[k]))
            return cps
        def out_copy(r0, nr, c0, w):
            return pltpu.make_async_copy(o_v.at[pl.ds(r0, nr), pl.ds(c0, w)], o_hbm.at[pl.ds(r0, nr), pl.ds(c0, w)], sems.at[0])

        for k in range(nst):
            for c in in_copies(k):
                c.start()

        A1 = []; A2 = []; B1 = {}; KDONE = {}

        def pw1(g0, g1):
            tc = slice(g0, g1); bc = slice(FH + g0, FH + g1)
            top = w1_v[:2 * KT, tc].T
            bot = w1_v[:2 * KT, bc].T
            a11, a12 = top[:, :KT], top[:, KT:]
            a21, a22 = bot[:, :KT], bot[:, KT:]
            a1, a2, a3 = w1_v[256:320, tc], w1_v[320:384, tc], w1_v[384:448, tc]
            d1, d2, d3 = w1_v[256:320, bc], w1_v[320:384, bc], w1_v[384:448, bc]
            at = jnp.concatenate([a1, sub(a2, d2)], axis=0).T
            ab = jnp.concatenate([d1, sub(d3, a3)], axis=0).T
            az = jnp.concatenate([d2, a3], axis=0).T
            lc = lambda u, v: jnp.concatenate([u, v], axis=1)
            A1.append((g0, g1, [add(a11, a22), add(a21, a22), lc(a11, az), lc(a22, az), add(a11, a12), lc(sub(a21, a11), ab), lc(sub(a12, a22), at), at, ab]))

        def pw2(g0, g1):
            a11 = w2t_v[:DH, g0:g1]; a12 = w2t_v[:DH, FH + g0:FH + g1]
            a21 = w2t_v[DH:, g0:g1]; a22 = w2t_v[DH:, FH + g0:FH + g1]
            A2.extend([add(a11, a22), add(a21, a22), a11, a22, add(a11, a12), sub(a21, a11), sub(a12, a22)])

        def px(j):
            s0, w = tstart[j], tiles[j] // 2
            b11 = xt_v[:KT, s0:s0 + w]; b12 = xt_v[:KT, s0 + w:s0 + 2 * w]
            b21 = xt_v[KT:2 * KT, s0:s0 + w]; b22 = xt_v[KT:2 * KT, s0 + w:s0 + 2 * w]
            L = slice(s0, s0 + w); R = slice(s0 + w, s0 + 2 * w)
            rc = lambda *u: jnp.concatenate(u, axis=0)
            B1[j] = [add(b11, b22), b11, rc(sub(b12, b22), xt_v[320:448, R]), rc(sub(b21, b11), xt_v[320:448, L]), b22,
                     rc(add(b11, b12), xt_v[256:320, R], xt_v[384:448, R]), rc(add(b21, b22), xt_v[256:384, L]),
                     xt_v[256:384, R], rc(xt_v[256:320, L], xt_v[384:448, L])]

        def mm1(g0, g1, j, order='std'):
            chunks = [(a0, a1, arrs) for (a0, a1, arrs) in sorted(A1, key=lambda t: t[0]) if g0 <= a0 and a1 <= g1]
            assert sum(c[1] - c[0] for c in chunks) == g1 - g0
            if bigfirst: chunks = sorted(chunks, key=lambda c: c[0] - c[1])
            for n, (c0, c1, arrs) in enumerate(chunks):
                mm1c(c0, c1, arrs, j, order if n == 0 else 'std')

        def mm1c(g0, g1, arrs, j, order):
            w = tiles[j] // 2
            m = [None] * 9
            for i in ORDS[order]:
                m[i] = dot(arrs[i], B1[j][i])
            m1, m2, m3, m4, m5, m6, m7, tr, bl = m
            h11 = act(m1 + m4 - m5 + m7)
            h12 = act(m3 + m5 + tr)
            h21 = act(m2 + m4 + bl)
            h22 = act(m1 - m2 + m3 + m6)
            vals = [(h11 + h22).astype(bf), h11.astype(bf), (h12 - h22).astype(bf), (h21 - h11).astype(bf),
                    h22.astype(bf), (h11 + h12).astype(bf), (h21 + h22).astype(bf)]
            c0 = tstart[j] // 2
            for i in (1, 5, 3, 0, 2, 4, 6):
                hs_v[i, g0:g1, c0:c0 + w] = vals[i]

        def mm2(j, order=None):
            order = order or order2
            s0, w = tstart[j], tiles[j] // 2
            c0h = s0 // 2
            acc = [None] * 7
            KDONE[j] = True
            final_op = lastsplit is not None and len(KDONE) == len(tiles)
            for n, i in enumerate(order):
                hh = hs_v[i, :, c0h:c0h + w]
                if final_op and n == 6:
                    assert i == 6
                    m1, m2, m3, m4, m5, m6, m7 = acc
                    nr, cw = lastsplit
                    rs = DH // nr
                    for c in range(0, w, cw):
                        for r in range(0, DH, rs):
                            sl = (slice(r, r + rs), slice(c, c + cw))
                            p = dot(A2[i][r:r + rs], hh[:, c:c + cw])
                            o_v[r:r + rs, s0 + c:s0 + c + cw] = (m1[sl] + m4[sl] - m5[sl] + p).astype(bf)
                            out_copy(r, rs, s0 + c, cw).start()
                    break
                acc[i] = dot(A2[i], hh)
                m1, m2, m3, m4, m5, m6, m7 = acc
                done = set(order[:n + 1])
                fin = lambda need: i in need and set(need) <= done
                for need, r0, c0, val in (((1, 3), DH, s0, lambda: m2 + m4),
                                          ((0, 1, 2, 5), DH, s0 + w, lambda: m1 - m2 + m3 + m6),
                                          ((2, 4), 0, s0 + w, lambda: m3 + m5),
                                          ((0, 3, 4, 6), 0, s0, lambda: m1 + m4 - m5 + m7)):
                    if fin(need):
                        o_v[r0:r0 + DH, c0:c0 + w] = val().astype(bf)
                        out_copy(r0, DH, c0, w).start()

        fns = dict(px=px, pw1=pw1, pw2=pw2, mm1=mm1, mm2=mm2)
        for k in range(nst):
            with scope(f"wait{k}"):
                for c in in_copies(k):
                    c.wait()
            with scope(f"stage{k}"):
                for op in plan[k][1]:
                    fns[op[0]](*op[1:])
        assert len(KDONE) == len(tiles)
        with scope("waitout"):
            pltpu.make_async_copy(o_v, o_hbm, sems.at[0]).wait()

    def fn(x, w1, w2):
        B = x.shape[0]
        xt = x.reshape(S, D).T
        w2t = w2.T
        out = pl.pallas_call(kernel,
            in_specs=[pl.BlockSpec(memory_space=pl.ANY)]*3,
            out_specs=pl.BlockSpec(memory_space=pl.ANY),
            out_shape=jax.ShapeDtypeStruct((D, S), x.dtype),
            scratch_shapes=[pltpu.VMEM((D, S + xpad), bf), pltpu.VMEM((D, F), bf), pltpu.VMEM((D, F), bf), pltpu.VMEM((D, S), bf),
                            pltpu.VMEM((7, FH, S // 2 + hpad), bf),
                            pltpu.SemaphoreType.DMA((nst,))],
            compiler_params=pltpu.CompilerParams(vmem_limit_bytes=120*1024*1024),
        )(xt, w1, w2t)
        return out.T.reshape(B, S, D)
    return fn

def auto(tiles, stages, o2first=(3, 2, 1, 5, 0, 4, 6), split0=True, wide2=True, **kw):
    nt = len(tiles)
    full = list(stages) + [(nt, FH)]
    if split0:
        full = [(0, full[0][1])] + full
    plan = []
    for k, (t1, g1) in enumerate(full):
        t0, g0 = (0, 0) if k == 0 else full[k - 1]
        loads = []
        if g1 > g0: loads.append(('w1', g0, g1))
        if t1 > t0: loads.append(('x', t0, t1))
        last = k == len(full) - 1
        if last: loads.append(('w2', 0, FH))
        ops = []
        newt = list(range(t0, t1)); oldt = list(range(0, t0))
        if not last:
            for n, j in enumerate(newt):
                ops.append(('px', j))
                if g0 > 0: ops.append(('mm1', 0, g0, j, 'nb' if n == 0 else 'std'))
            if g1 > g0:
                ops.append(('pw1', g0, g1))
                order = sorted(oldt + newt, key=lambda j: -tiles[j])
                for n, j in enumerate(order):
                    ops.append(('mm1', g0, g1, j, 'na' if n == 0 else 'std'))
        else:
            first = newt[0] if newt else None
            done1 = set()
            if first is not None:
                ops += [('px', first), ('mm1', 0, g0, first, 'nb')]
            if g1 > g0: ops.append(('pw1', g0, g1))
            ops.append(('pw2', 0, FH))
            if g1 > g0 and first is not None:
                ops.append(('mm1', g0, g1, first, 'na')); done1.add(first)
            n2 = 0
            torder = list(range(nt))
            if wide2 and first is not None:
                torder.remove(first)
                if g1 > g0:
                    j0 = torder[0]
                    ops.append(('mm1', g0, g1, j0)); done1.add(j0)
                torder = [first] + torder
            for j in torder:
                if j not in done1:
                    if j in newt and j != first:
                        ops += [('px', j), ('mm1', 0, FH, j)]
                    elif g1 > g0:
                        ops.append(('mm1', g0, g1, j))
                ops.append(('mm2', j) + ((o2first,) if n2 == 0 else ()))
                n2 += 1
        plan.append((loads, ops))
    return make(tuple(tiles), plan, **kw)


_impl = auto((256,256,512,512,512),[(1,128),(2,256),(3,384),(4,896)])


@jax.jit
def pallas_standalone__dense_activation_silu__prompt_kernel(x, w1, w2):
    return _impl(x, w1, w2)
```

```python
import contextlib
import jax, jax.numpy as jnp
from jax.experimental import pallas as pl
from jax.experimental.pallas import tpu as pltpu
D, S, F = 448, 2048, 1792
KT = 128; FH = F // 2; DH = D // 2
bf = jnp.bfloat16; f32 = jnp.float32

def dot(a, b): return jnp.dot(a, b, preferred_element_type=f32)
def add(u, v): return (u.astype(f32) + v.astype(f32)).astype(bf)
def sub(u, v): return (u.astype(f32) - v.astype(f32)).astype(bf)
def act(h):
    hh = 0.5 * h
    return hh + hh * jnp.tanh(hh)

ORD = dict(std=(0, 3, 4, 7, 6, 2, 8, 1, 5),
           nb=(7, 4, 3, 0, 6, 2, 8, 1, 5),
           na=(3, 2, 7, 4, 0, 6, 8, 1, 5))

def make(tiles, plan, scopes=False, xpad=128, order2=(1, 3, 5, 0, 2, 4, 6), hpad=128, lastsplit=(2, 128), bigfirst=True, ords=None):
    assert sum(tiles) == S
    tstart = [sum(tiles[:i]) for i in range(len(tiles) + 1)]
    nst = len(plan)
    scope = (lambda n: jax.named_scope(n)) if scopes else (lambda n: contextlib.nullcontext())
    ORDS = dict(ORD); ORDS.update(ords or {})

    def kernel(xt_hbm, w1_hbm, w2t_hbm, o_hbm, xt_v, w1_v, w2t_v, o_v, hs_v, sems):
        def in_copies(k):
            cps = []
            for ld in plan[k][0]:
                if ld[0] in ('w1', 'w2'):
                    src, dst = (w1_hbm, w1_v) if ld[0] == 'w1' else (w2t_hbm, w2t_v)
                    g0, g1 = ld[1:]
                    if g0 == 0 and g1 == FH:
                        cps.append(pltpu.make_async_copy(src, dst, sems.at[k]))
                    else:
                        for off in (0, FH):
                            cps.append(pltpu.make_async_copy(src.at[:, pl.ds(off + g0, g1 - g0)], dst.at[:, pl.ds(off + g0, g1 - g0)], sems.at[k]))
                elif ld[0] == 'x':
                    s0, s1 = tstart[ld[1]], tstart[ld[2]]
                    cps.append(pltpu.make_async_copy(xt_hbm.at[:, pl.ds(s0, s1 - s0)], xt_v.at[:, pl.ds(s0, s1 - s0)], sems.at[k]))
            return cps
        def out_copy(r0, nr, c0, w):
            return pltpu.make_async_copy(o_v.at[pl.ds(r0, nr), pl.ds(c0, w)], o_hbm.at[pl.ds(r0, nr), pl.ds(c0, w)], sems.at[0])

        for k in range(nst):
            for c in in_copies(k):
                c.start()
        hs_v[0:8, S:S + 128] = jnp.zeros((8, 128), f32)
        pin = pltpu.make_async_copy(hs_v.at[pl.ds(0, 8), pl.ds(S, 128)], hs_v.at[pl.ds(8, 8), pl.ds(S, 128)], sems.at[nst - 1])
        pin.start()

        A1 = []; A2 = []; B1 = {}; KDONE = {}

        def pw1(g0, g1):
            tc = slice(g0, g1); bc = slice(FH + g0, FH + g1)
            top = w1_v[:2 * KT, tc].T
            bot = w1_v[:2 * KT, bc].T
            a11, a12 = top[:, :KT], top[:, KT:]
            a21, a22 = bot[:, :KT], bot[:, KT:]
            a1, a2, a3 = w1_v[256:320, tc], w1_v[320:384, tc], w1_v[384:448, tc]
            d1, d2, d3 = w1_v[256:320, bc], w1_v[320:384, bc], w1_v[384:448, bc]
            at = jnp.concatenate([a1, sub(a2, d2)], axis=0).T
            ab = jnp.concatenate([d1, sub(d3, a3)], axis=0).T
            az = jnp.concatenate([d2, a3], axis=0).T
            lc = lambda u, v: jnp.concatenate([u, v], axis=1)
            A1.append((g0, g1, [add(a11, a22), add(a21, a22), lc(a11, az), lc(a22, az), add(a11, a12), lc(sub(a21, a11), ab), lc(sub(a12, a22), at), at, ab]))

        def pw2(g0, g1):
            if l2:
                for i in range(7 if eager else 0):
                    for q in range(7):
                        a2l2(i, q)
                return
            a11 = w2t_v[:DH, g0:g1]; a12 = w2t_v[:DH, FH + g0:FH + g1]
            a21 = w2t_v[DH:, g0:g1]; a22 = w2t_v[DH:, FH + g0:FH + g1]
            A2.extend([add(a11, a22), add(a21, a22), a11, a22, add(a11, a12), sub(a21, a11), sub(a12, a22)])

        SA = [((1, 0, 0), (1, 1, 1)), ((1, 1, 0), (1, 1, 1)), ((1, 0, 0),), ((1, 1, 1),), ((1, 0, 0), (1, 0, 1)), ((1, 1, 0), (-1, 0, 0)), ((1, 0, 1), (-1, 1, 1))]
        SB = [((1, 0, 0), (1, 1, 1)), ((1, 0, 0),), ((1, 0, 1), (-1, 1, 1)), ((1, 1, 0), (-1, 0, 0)), ((1, 1, 1),), ((1, 0, 0), (1, 0, 1)), ((1, 1, 0), (1, 1, 1))]
        KS = 384; DQ = DH // 2
        def lin(terms, get):
            acc = None
            for (c, u, v) in terms:
                t = get(u, v)
                acc = t if acc is None else (acc + t if c > 0 else acc - t)
            return acc
        def lin2(to, ti, get):
            terms = [(co * ci, uo, vo, ui, vi) for (co, uo, vo) in to for (ci, ui, vi) in ti]
            if len(terms) == 4:
                terms = [terms[0], terms[3], terms[1], terms[2]]
            acc = None
            for (c, uo, vo, ui, vi) in terms:
                t = get(uo, vo, ui, vi)
                if acc is None:
                    assert c > 0
                    acc = t
                else:
                    acc = acc + t if c > 0 else acc - t
            return acc
        A22 = {}; A21 = {}
        def a2l2(i, q):
            if (i, q) not in A22:
                outer = lambda r0, nr, k0, nk: lin(SA[i], lambda r, k: w2t_v[r * DH + r0:r * DH + r0 + nr, k * FH + k0:k * FH + k0 + nk].astype(f32))
                if flat_a:
                    main = lin2(SA[i], SA[q], lambda r, k, r2, k2: w2t_v[r * DH + r2 * DQ:r * DH + (r2 + 1) * DQ, k * FH + k2 * KS:k * FH + (k2 + 1) * KS].astype(f32))
                else:
                    main = lin(SA[q], lambda r, k: outer(r * DQ, DQ, k * KS, KS))
                ar = lambda r: outer(r * DQ, DQ, 2 * KS, KT)
                extra = {2: lambda: ar(0), 5: lambda: ar(1) - ar(0), 3: lambda: ar(1), 6: lambda: ar(0) - ar(1)}.get(q)
                if extra is not None:
                    main = jnp.concatenate([main, extra()], axis=1)
                A22[(i, q)] = main.astype(bf)
            return A22[(i, q)]

        GEN = {}
        def mm2l2(s0, W2, order=None, last=False, nsteps=7):
            if s0 not in GEN:
                GEN[s0] = mm2gen(s0, W2, order, last)
            for _ in range(nsteps):
                next(GEN[s0])

        def mm2gen(s0, W2, order=None, last=False):
            order = order or order2
            w = W2 // 2; wq = w // 2
            P = [None] * 7
            def b2l2(i, q):
                outer = lambda k0, nk, c0: lin(SB[i], lambda k, c: hs_v[k * FH + k0:k * FH + k0 + nk, s0 + c * w + c0:s0 + c * w + c0 + wq])
                if flat_b:
                    main = lin2(SB[i], SB[q], lambda k, c, k2, c2: hs_v[k * FH + k2 * KS:k * FH + (k2 + 1) * KS, s0 + c * w + c2 * wq:s0 + c * w + (c2 + 1) * wq])
                else:
                    main = lin(SB[q], lambda k, c: outer(k * KS, KS, c * wq))
                cx = {2: 1, 5: 1, 3: 0, 6: 0}.get(q)
                if cx is not None:
                    main = jnp.concatenate([main, outer(2 * KS, KT, cx * wq)], axis=0)
                return main.astype(bf)
            CN = {(0, 0): ((1, 0), (1, 3), (-1, 4), (1, 6)), (0, 1): ((1, 2), (1, 4)), (1, 0): ((1, 1), (1, 3)), (1, 1): ((1, 0), (-1, 1), (1, 2), (1, 5))}
            def comb(ms, key):
                acc = None
                for (c, t) in CN[key]:
                    acc = ms[t] if acc is None else (acc + ms[t] if c > 0 else acc - ms[t])
                return acc
            for n, i in enumerate(order):
                ms = [None] * 7
                P[i] = {}
                done_o = set(order[:n + 1])
                if i not in l2set:
                    if i not in A21:
                        A21[i] = lin(SA[i], lambda r, k: w2t_v[r * DH:(r + 1) * DH, k * FH:(k + 1) * FH].astype(f32)).astype(bf)
                    gi = lin(SB[i], lambda k, c: hs_v[k * FH:(k + 1) * FH, s0 + c * w:s0 + (c + 1) * w]).astype(bf)
                    split = last and n == 6
                    if not split:
                        full = dot(A21[i], gi)
                    for key in ((1, 0), (1, 1), (0, 1), (0, 0)):
                        rs = slice(key[0] * DQ, (key[0] + 1) * DQ); cs = slice(key[1] * wq, (key[1] + 1) * wq)
                        P[i][key] = dot(A21[i][rs], gi[:, cs]) if split else full[rs, cs]
                        for okey, oterms in CN.items():
                            oneed = {t for _, t in oterms}
                            if i in oneed and oneed <= done_o:
                                val = comb([None if p is None else p.get(key) for p in P], okey)
                                r0 = okey[0] * DH + key[0] * DQ; c0 = s0 + okey[1] * w + key[1] * wq
                                o_v[r0:r0 + DQ, c0:c0 + wq] = val.astype(bf)
                                if split:
                                    out_copy(r0, DQ, c0, wq).start()
                for nq, q in enumerate(inner2 if i in l2set else ()):
                    ms[q] = dot(a2l2(i, q), b2l2(i, q))
                    done = set(inner2[:nq + 1])
                    for key, terms in CN.items():
                        need = {t for _, t in terms}
                        if q in need and need <= done:
                            P[i][key] = comb(ms, key)
                            for okey, oterms in CN.items():
                                oneed = {t for _, t in oterms}
                                if i in oneed and oneed <= done_o:
                                    val = comb([None if p is None else p.get(key) for p in P], okey)
                                    r0 = okey[0] * DH + key[0] * DQ; c0 = s0 + okey[1] * w + key[1] * wq
                                    o_v[r0:r0 + DQ, c0:c0 + wq] = val.astype(bf)
                                    if last and n == 6:
                                        out_copy(r0, DQ, c0, wq).start()
                if not (last and n == 6):
                    for okey, oterms in CN.items():
                        oneed = {t for _, t in oterms}
                        if i in oneed and oneed <= done_o:
                            out_copy(okey[0] * DH, DH, s0 + okey[1] * w, w).start()
                yield

        def px(j):
            s0, w = tstart[j], tiles[j] // 2
            b11 = xt_v[:KT, s0:s0 + w]; b12 = xt_v[:KT, s0 + w:s0 + 2 * w]
            b21 = xt_v[KT:2 * KT, s0:s0 + w]; b22 = xt_v[KT:2 * KT, s0 + w:s0 + 2 * w]
            L = slice(s0, s0 + w); R = slice(s0 + w, s0 + 2 * w)
            rc = lambda *u: jnp.concatenate(u, axis=0)
            B1[j] = [add(b11, b22), b11, rc(sub(b12, b22), xt_v[320:448, R]), rc(sub(b21, b11), xt_v[320:448, L]), b22,
                     rc(add(b11, b12), xt_v[256:320, R], xt_v[384:448, R]), rc(add(b21, b22), xt_v[256:384, L]),
                     xt_v[256:384, R], rc(xt_v[256:320, L], xt_v[384:448, L])]

        def mm1(g0, g1, j, order='std'):
            chunks = [(a0, a1, arrs) for (a0, a1, arrs) in sorted(A1, key=lambda t: t[0]) if g0 <= a0 and a1 <= g1]
            assert sum(c[1] - c[0] for c in chunks) == g1 - g0
            if bigfirst: chunks = sorted(chunks, key=lambda c: c[0] - c[1])
            for n, (c0, c1, arrs) in enumerate(chunks):
                mm1c(c0, c1, arrs, j, order if n == 0 else 'std')

        def mm1c(g0, g1, arrs, j, order):
            w = tiles[j] // 2
            m = [None] * 9
            for i in ORDS[order]:
                m[i] = dot(arrs[i], B1[j][i])
            m1, m2, m3, m4, m5, m6, m7, tr, bl = m
            h11 = act(m1 + m4 - m5 + m7)
            h12 = act(m3 + m5 + tr)
            h21 = act(m2 + m4 + bl)
            h22 = act(m1 - m2 + m3 + m6)
            s0 = tstart[j]
            hs_v[g0:g1, s0:s0 + w] = h11
            hs_v[g0:g1, s0 + w:s0 + 2 * w] = h12
            hs_v[FH + g0:FH + g1, s0:s0 + w] = h21
            hs_v[FH + g0:FH + g1, s0 + w:s0 + 2 * w] = h22

        def mm2(j, order=None):
            if l2:
                KDONE[j] = True
                return mm2l2(tstart[j], tiles[j], order, len(KDONE) == len(tiles))
            order = order or order2
            s0, w = tstart[j], tiles[j] // 2
            c0h = s0 // 2
            acc = [None] * 7
            KDONE[j] = True
            final_op = lastsplit is not None and len(KDONE) == len(tiles)
            for n, i in enumerate(order):
                H = lambda a, b: hs_v[a * FH:(a + 1) * FH, s0 + b * w:s0 + (b + 1) * w]
                hh = [lambda: H(0, 0) + H(1, 1), lambda: H(0, 0), lambda: H(0, 1) - H(1, 1), lambda: H(1, 0) - H(0, 0),
                      lambda: H(1, 1), lambda: H(0, 0) + H(0, 1), lambda: H(1, 0) + H(1, 1)][i]().astype(bf)
                if final_op and n == 6:
                    assert i == 6
                    m1, m2, m3, m4, m5, m6, m7 = acc
                    nr, cw = lastsplit
                    rs = DH // nr
                    for c in range(0, w, cw):
                        for r in range(0, DH, rs):
                            sl = (slice(r, r + rs), slice(c, c + cw))
                            p = dot(A2[i][r:r + rs], hh[:, c:c + cw])
                            o_v[r:r + rs, s0 + c:s0 + c + cw] = (m1[sl] + m4[sl] - m5[sl] + p).astype(bf)
                            out_copy(r, rs, s0 + c, cw).start()
                    break
                acc[i] = dot(A2[i], hh)
                m1, m2, m3, m4, m5, m6, m7 = acc
                done = set(order[:n + 1])
                fin = lambda need: i in need and set(need) <= done
                for need, r0, c0, val in (((1, 3), DH, s0, lambda: m2 + m4),
                                          ((0, 1, 2, 5), DH, s0 + w, lambda: m1 - m2 + m3 + m6),
                                          ((2, 4), 0, s0 + w, lambda: m3 + m5),
                                          ((0, 3, 4, 6), 0, s0, lambda: m1 + m4 - m5 + m7)):
                    if fin(need):
                        o_v[r0:r0 + DH, c0:c0 + w] = val().astype(bf)
                        out_copy(r0, DH, c0, w).start()

        fns = dict(mm2w=mm2l2, px=px, pw1=pw1, pw2=pw2, mm1=mm1, mm2=mm2)
        for k in range(nst):
            with scope(f"wait{k}"):
                for c in in_copies(k):
                    c.wait()
                if k == nst - 1:
                    pin.wait()
            with scope(f"stage{k}"):
                for op in plan[k][1]:
                    fns[op[0]](*op[1:])
        with scope("waitout"):
            pltpu.make_async_copy(o_v, o_hbm, sems.at[0]).wait()

    def fn(x, w1, w2):
        B = x.shape[0]
        xt = x.reshape(S, D).T
        w2t = w2.T
        out = pl.pallas_call(kernel,
            in_specs=[pl.BlockSpec(memory_space=pl.ANY)]*3,
            out_specs=pl.BlockSpec(memory_space=pl.ANY),
            out_shape=jax.ShapeDtypeStruct((D, S), x.dtype),
            scratch_shapes=[pltpu.VMEM((D, S + xpad), bf), pltpu.VMEM((D, F), bf), pltpu.VMEM((D, F), bf), pltpu.VMEM((D, S), bf),
                            pltpu.VMEM((F, S + hpad), f32),
                            pltpu.SemaphoreType.DMA((nst,))],
            compiler_params=pltpu.CompilerParams(vmem_limit_bytes=120*1024*1024),
        )(xt, w1, w2t)
        return out.T.reshape(B, S, D)
    return fn

def auto(tiles, stages, o2first=(3, 2, 1, 5, 0, 4, 6), split0=True, wide2=True, **kw):
    nt = len(tiles)
    full = list(stages) + [(nt, FH)]
    if split0:
        full = [(0, full[0][1])] + full
    plan = []
    for k, (t1, g1) in enumerate(full):
        t0, g0 = (0, 0) if k == 0 else full[k - 1]
        loads = []
        if g1 > g0: loads.append(('w1', g0, g1))
        if t1 > t0: loads.append(('x', t0, t1))
        last = k == len(full) - 1
        if last: loads.append(('w2', 0, FH))
        ops = []
        newt = list(range(t0, t1)); oldt = list(range(0, t0))
        if not last:
            for n, j in enumerate(newt):
                ops.append(('px', j))
                if g0 > 0: ops.append(('mm1', 0, g0, j, 'nb' if n == 0 else 'std'))
            if g1 > g0:
                ops.append(('pw1', g0, g1))
                order = sorted(oldt + newt, key=lambda j: -tiles[j])
                for n, j in enumerate(order):
                    ops.append(('mm1', g0, g1, j, 'na' if n == 0 else 'std'))
        else:
            first = newt[0] if newt else None
            done1 = set()
            if first is not None:
                ops += [('px', first), ('mm1', 0, g0, first, 'nb')]
            if g1 > g0: ops.append(('pw1', g0, g1))
            ops.append(('pw2', 0, FH))
            if g1 > g0 and first is not None:
                ops.append(('mm1', g0, g1, first, 'na')); done1.add(first)
            n2 = 0
            torder = list(range(nt))
            if wide2 and first is not None:
                torder.remove(first)
                if g1 > g0:
                    j0 = torder[0]
                    ops.append(('mm1', g0, g1, j0)); done1.add(j0)
                torder = [first] + torder
            for j in torder:
                if j not in done1:
                    if j in newt and j != first:
                        ops += [('px', j), ('mm1', 0, FH, j)]
                    elif g1 > g0:
                        ops.append(('mm1', g0, g1, j))
                ops.append(('mm2', j) + ((o2first,) if n2 == 0 else ()))
                n2 += 1
        plan.append((loads, ops))
    return make(tuple(tiles), plan, **kw)


def planW(v=0, **kw):
    T = (512, 512, 512, 512)
    s0 = ([('w1', 0, 128)], [('pw1', 0, 128)])
    s1 = ([('x', 0, 1)], [('px', 0), ('mm1', 0, 128, 0, 'nb')])
    s2 = ([('w1', 128, 384)], [('pw1', 128, 384), ('mm1', 128, 384, 0, 'na')])
    s3 = ([('w1', 384, 640), ('x', 1, 2)], [('px', 1), ('mm1', 0, 384, 1, 'nb'), ('pw1', 384, 640), ('mm1', 384, 640, 0, 'na'), ('mm1', 384, 640, 1)])
    if v == 0:
        s4 = ([('w1', 640, 896), ('x', 2, 3), ('w2', 0, 896)], [('px', 2), ('mm1', 0, 640, 2, 'nb'), ('pw1', 640, 896), ('pw2', 0, 896), ('mm1', 640, 896, 2, 'na'), ('mm1', 640, 896, 0), ('mm1', 640, 896, 1)])
        s5 = ([('x', 3, 4)], [('mm2', 0), ('px', 3), ('mm1', 0, 896, 3), ('mm2', 1), ('mm2', 2), ('mm2', 3)])
        plan = [s0, s1, s2, s3, s4, s5]
    if v == 1:
        s4 = ([('w1', 640, 896), ('x', 2, 4), ('w2', 0, 896)], [('px', 2), ('mm1', 0, 640, 2, 'nb'), ('pw1', 640, 896), ('pw2', 0, 896), ('mm1', 640, 896, 2, 'na'), ('mm1', 640, 896, 0), ('mm1', 640, 896, 1), ('px', 3), ('mm1', 0, 896, 3)])
        s5 = ([], [('mm2', 0), ('mm2', 1), ('mm2', 2), ('mm2', 3)])
        plan = [s0, s1, s2, s3, s4, s5]
    return make(T, plan, **kw)


def planX(W2=2048, o2=None, **kw):
    T = (512, 512, 512, 512)
    s0 = ([('w1', 0, 128)], [('pw1', 0, 128)])
    s1 = ([('x', 0, 1)], [('px', 0), ('mm1', 0, 128, 0, 'nb')])
    s2 = ([('w1', 128, 384)], [('pw1', 128, 384), ('mm1', 128, 384, 0, 'na')])
    s3 = ([('w1', 384, 640), ('x', 1, 2)], [('px', 1), ('mm1', 0, 384, 1, 'nb'), ('pw1', 384, 640), ('mm1', 384, 640, 0, 'na'), ('mm1', 384, 640, 1)])
    ops = [('px', 2), ('mm1', 0, 640, 2, 'nb'), ('pw1', 640, 896), ('mm1', 640, 896, 2, 'na'), ('mm1', 640, 896, 0), ('mm1', 640, 896, 1), ('px', 3), ('mm1', 0, 896, 3)]
    for s in range(0, S, W2):
        ops.append(('mm2w', s, W2, o2, s + W2 == S))
    s4 = ([('w1', 640, 896), ('x', 2, 4), ('w2', 0, 896)], ops)
    return make(T, [s0, s1, s2, s3, s4], **kw)


def planY(v=0, o2=(3, 2, 1, 5, 0, 4, 6), **kw):
    T = (512, 512, 512, 512)
    s0 = ([('w1', 0, 128)], [('pw1', 0, 128)])
    s1 = ([('x', 0, 1)], [('px', 0), ('mm1', 0, 128, 0, 'nb')])
    s2 = ([('w1', 128, 384)], [('pw1', 128, 384), ('mm1', 128, 384, 0, 'na')])
    s3 = ([('w1', 384, 640), ('x', 1, 2)], [('px', 1), ('mm1', 0, 384, 1, 'nb'), ('pw1', 384, 640), ('mm1', 384, 640, 0, 'na'), ('mm1', 384, 640, 1)])
    P = lambda t, n, last=False: ('mm2w', 512 * t, 512, o2 if t == 0 else None, last, n)
    if v == 0:
        ops = [('px', 2), ('mm1', 128, 384, 2, 'nb'), ('pw1', 640, 896), ('mm1', 640, 896, 0, 'na'), ('mm1', 384, 640, 2),
               P(0, 2), ('mm1', 640, 896, 1), P(0, 1), ('mm1', 640, 896, 2), P(0, 1), ('mm1', 0, 128, 2), ('px', 3), P(0, 1), ('mm1', 128, 384, 3), P(0, 1), ('mm1', 384, 640, 3), P(0, 1),
               ('mm1', 640, 896, 3), ('mm1', 0, 128, 3), P(1, 7), P(2, 7), P(3, 7, True)]
    if v == 1:
        ops = [('px', 2), ('mm1', 128, 384, 2, 'nb'), ('pw1', 640, 896), ('mm1', 640, 896, 0, 'na'), ('mm1', 384, 640, 2),
               P(0, 2), ('mm1', 640, 896, 1), P(0, 1), ('mm1', 640, 896, 2), P(0, 1), ('mm1', 0, 128, 2), P(1, 2), P(0, 1), P(1, 2), P(0, 1), P(1, 2), P(0, 1), P(1, 1),
               ('px', 3), ('mm1', 0, 896, 3), P(2, 7), P(3, 7, True)]
    s4 = ([('w1', 640, 896), ('x', 2, 4), ('w2', 0, 896)], ops)
    return make(T, [s0, s1, s2, s3, s4], **kw)


def planZ(v=0, of=(3, 5, 2, 0, 1, 6, 4), om=(1, 5, 3, 0, 2, 6, 4), ol=(1, 5, 3, 0, 2, 4, 6), **kw):
    kw.setdefault('l2set', (1, 2, 3, 4))
    T = (512, 512, 512, 512)
    s0 = ([('w1', 0, 128)], [('pw1', 0, 128)])
    s1 = ([('x', 0, 1)], [('px', 0), ('mm1', 0, 128, 0, 'nb')])
    s2 = ([('w1', 128, 384)], [('pw1', 128, 384), ('mm1', 128, 384, 0, 'na')])
    s3 = ([('w1', 384, 640), ('x', 1, 2)], [('px', 1), ('mm1', 0, 384, 1, 'nb'), ('pw1', 384, 640), ('mm1', 384, 640, 0, 'na'), ('mm1', 384, 640, 1)])
    P = lambda t, n, o=None, last=False: ('mm2w', 512 * t, 512, o, last, n)
    pre = [('px', 2), ('mm1', 0, 640, 2, 'nb'), ('pw1', 640, 896), ('mm1', 640, 896, 2, 'na'), ('mm1', 640, 896, 0)]
    if v == 0:
        ops = pre + [P(2, 7, of), P(0, 7, om), ('mm1', 640, 896, 1), P(1, 7, om), ('px', 3), ('mm1', 0, 896, 3), P(3, 7, ol, True)]
    if v == 1:
        ops = pre + [P(2, 4, of), ('mm1', 640, 896, 1), P(2, 2), ('px', 3), ('mm1', 128, 384, 3), P(2, 1), P(0, 7, om), ('mm1', 384, 640, 3), P(1, 7, om),
                     ('mm1', 640, 896, 3), ('mm1', 0, 128, 3), P(3, 7, ol, True)]
    if v == 2:
        ops = pre + [P(2, 4, of), P(0, 2, of), P(2, 1), P(0, 2), P(2, 2), P(0, 3), ('mm1', 640, 896, 1), P(1, 7, om), ('px', 3), ('mm1', 0, 896, 3), P(3, 7, ol, True)]
    if v == 3:
        ops = pre + [P(2, 1, of), P(0, 1, of), P(2, 1), P(0, 1), P(2, 1), P(0, 1), P(2, 1), P(0, 1), P(2, 1), P(0, 1), P(2, 1), P(0, 1), P(2, 1), P(0, 1),
                     ('mm1', 640, 896, 1), P(1, 7, om), ('px', 3), ('mm1', 0, 896, 3), P(3, 7, ol, True)]
    s4 = ([('w1', 640, 896), ('x', 2, 4), ('w2', 0, 896)], ops)
    return make(T, [s0, s1, s2, s3, s4], **kw)


_impl = planZ(3)


@jax.jit
def pallas_standalone__dense_activation_silu__prompt_kernel(x, w1, w2):
    return _impl(x, w1, w2)
```

```python
import contextlib
import jax, jax.numpy as jnp
from jax.experimental import pallas as pl
from jax.experimental.pallas import tpu as pltpu
D, S, F = 448, 2048, 1792
KT = 128; FH = F // 2; DH = D // 2; DQ = D // 4; KS = 384
bf = jnp.bfloat16; f32 = jnp.float32

def dot(a, b): return jnp.dot(a, b, preferred_element_type=f32)
def add(u, v): return (u.astype(f32) + v.astype(f32)).astype(bf)
def sub(u, v): return (u.astype(f32) - v.astype(f32)).astype(bf)
def act(h):
    hh = 0.5 * h
    return hh + hh * jnp.tanh(hh)

ORD = dict(std=(0, 3, 4, 6, 2, 1, 5),
           nb=(1, 4, 3, 0, 6, 2, 5),
           na=(2, 3, 4, 0, 6, 1, 5))
SA = [((1, 0, 0), (1, 1, 1)), ((1, 1, 0), (1, 1, 1)), ((1, 0, 0),), ((1, 1, 1),), ((1, 0, 0), (1, 0, 1)), ((1, 1, 0), (-1, 0, 0)), ((1, 0, 1), (-1, 1, 1))]
SB = [((1, 0, 0), (1, 1, 1)), ((1, 0, 0),), ((1, 0, 1), (-1, 1, 1)), ((1, 1, 0), (-1, 0, 0)), ((1, 1, 1),), ((1, 0, 0), (1, 0, 1)), ((1, 1, 0), (1, 1, 1))]
CN = {(0, 0): ((1, 0), (1, 3), (-1, 4), (1, 6)), (0, 1): ((1, 2), (1, 4)), (1, 0): ((1, 1), (1, 3)), (1, 1): ((1, 0), (-1, 1), (1, 2), (1, 5))}

def lin(terms, get):
    acc = None
    for (c, u, v) in terms:
        t = get(u, v)
        acc = t if acc is None else (acc + t if c > 0 else acc - t)
    return acc

def comb(ms, key):
    acc = None
    for (c, t) in CN[key]:
        acc = ms[t] if acc is None else (acc + ms[t] if c > 0 else acc - ms[t])
    return acc

def make(plan, scopes=False, xpad=128, hpad=128, inner2=(1, 3, 5, 0, 2, 4, 6), l2set=(1, 2, 3, 4), ords=None, l1set=(1, 2, 3, 4), inner1=(0, 3, 4, 6, 2, 1, 5)):
    nst = len(plan)
    scope = (lambda n: jax.named_scope(n)) if scopes else (lambda n: contextlib.nullcontext())
    ORDS = dict(ORD); ORDS.update(ords or {})

    def kernel(xt_hbm, w1_hbm, w2t_hbm, o_hbm, xt_v, w1_v, w2t_v, o_v, hs_v, sems):
        bufs = dict(x=(xt_hbm, xt_v), w1=(w1_hbm, w1_v), w2=(w2t_hbm, w2t_v))
        def in_copies(k):
            cps = []
            for (name, c0, c1) in plan[k][0]:
                src, dst = bufs[name]
                cps.append(pltpu.make_async_copy(src.at[:, pl.ds(c0, c1 - c0)], dst.at[:, pl.ds(c0, c1 - c0)], sems.at[k]))
            return cps
        outs = []
        def out_copy(r0, nr, c0, w):
            cp = pltpu.make_async_copy(o_v.at[pl.ds(r0, nr), pl.ds(c0, w)], o_hbm.at[pl.ds(r0, nr), pl.ds(c0, w)], sems.at[0])
            cp.start()
            outs.append(cp)

        for k in range(nst):
            for c in in_copies(k):
                c.start()
        hs_v[0:8, S:S + 128] = jnp.zeros((8, 128), f32)
        pin = pltpu.make_async_copy(hs_v.at[pl.ds(0, 8), pl.ds(S, 128)], hs_v.at[pl.ds(8, 8), pl.ds(S, 128)], sems.at[nst - 1])
        pin.start()

        A1 = {}; B1 = {}; A22 = {}; A21 = {}; GEN = {}
        cover = []

        def pw1(f0, nf):
            if (f0, nf) in A1: return A1[(f0, nf)]
            g = nf // 2
            tc = slice(f0, f0 + g); bc = slice(f0 + g, f0 + nf)
            top = w1_v[:2 * KT, tc].T
            bot = w1_v[:2 * KT, bc].T
            a11, a12 = top[:, :KT], top[:, KT:]
            a21, a22 = bot[:, :KT], bot[:, KT:]
            a1, a2, a3 = w1_v[256:320, tc], w1_v[320:384, tc], w1_v[384:448, tc]
            d1, d2, d3 = w1_v[256:320, bc], w1_v[320:384, bc], w1_v[384:448, bc]
            at = jnp.concatenate([a1, sub(a2, d2)], axis=0).T
            ab = jnp.concatenate([d1, sub(d3, a3)], axis=0).T
            az = jnp.concatenate([d2, a3], axis=0).T
            up = lambda u: u.astype(f32)
            halves = [None, (lambda: up(a21) + up(a22), ab), (lambda: a11, az), (lambda: a22, az), (lambda: up(a11) + up(a12), at),
                      (lambda: up(a21) - up(a11), ab), (lambda: up(a12) - up(a22), at)]
            res = [add(a11, a22)]
            for i in range(1, 7):
                k0 = halves[i][0](); k1 = halves[i][1]
                if i in l1set:
                    gh = g // 2
                    blk = lambda r, k: up((k0, k1)[k][r * gh:(r + 1) * gh])
                    res.append([lin(SA[q], blk).astype(bf) for q in range(7)])
                else:
                    res.append(jnp.concatenate([k0.astype(bf), k1], axis=1))
            A1[(f0, nf)] = res
            return res

        def px(s0, ns):
            if (s0, ns) in B1: return B1[(s0, ns)]
            w = ns // 2
            L = slice(s0, s0 + w); R = slice(s0 + w, s0 + ns)
            b11 = xt_v[:KT, L]; b12 = xt_v[:KT, R]
            b21 = xt_v[KT:2 * KT, L]; b22 = xt_v[KT:2 * KT, R]
            rc = lambda *u: jnp.concatenate(u, axis=0)
            up = lambda u: u.astype(f32)
            lr = lambda r0, r1: add(xt_v[r0:r1, L], xt_v[r0:r1, R])
            halves = [None, (lambda: b11, lambda: rc(xt_v[256:320, L], xt_v[384:448, L])), (lambda: up(b12) - up(b22), lambda: xt_v[320:448, R]),
                      (lambda: up(b21) - up(b11), lambda: xt_v[320:448, L]), (lambda: b22, lambda: xt_v[256:384, R]),
                      (lambda: lr(0, 128), lambda: rc(lr(256, 320), lr(384, 448))), (lambda: lr(128, 256), lambda: lr(256, 384))]
            res = [add(b11, b22)]
            for i in range(1, 7):
                k0 = halves[i][0](); k1 = halves[i][1]()
                if i in l1set:
                    wh = w // 2
                    blk = lambda k, c: up((k0, k1)[k][:, c * wh:(c + 1) * wh])
                    res.append([lin(SB[q], blk).astype(bf) for q in range(7)])
                else:
                    res.append(rc(k0.astype(bf), k1))
            B1[(s0, ns)] = res
            return B1[(s0, ns)]

        def mm1(f0, nf, s0, ns, order='std'):
            A = pw1(f0, nf); B = px(s0, ns)
            g = nf // 2; w = ns // 2
            cover.append(nf * ns)
            m = [None] * 7
            for i in ORDS[order]:
                if i == 0:
                    np_ = max(1, 4 // (w // 128))
                    rs = g // np_
                    m[i] = jnp.concatenate([dot(A[i][r:r + rs], B[i]) for r in range(0, g, rs)], axis=0)
                elif i in l1set:
                    ms = [None] * 7
                    for q in inner1:
                        ms[q] = dot(A[i][q], B[i][q])
                    m[i] = jnp.concatenate([jnp.concatenate([comb(ms, (r, c)) for c in range(2)], axis=1) for r in range(2)], axis=0)
                else:
                    m[i] = dot(A[i], B[i])
            m1, m2, m3, m4, m5, m6, m7 = m
            hs_v[f0:f0 + g, s0:s0 + w] = act(m1 + m4 - m5 + m7)
            hs_v[f0:f0 + g, s0 + w:s0 + ns] = act(m3 + m5)
            hs_v[f0 + g:f0 + nf, s0:s0 + w] = act(m2 + m4)
            hs_v[f0 + g:f0 + nf, s0 + w:s0 + ns] = act(m1 - m2 + m3 + m6)

        def a2l2(i, q):
            if (i, q) not in A22:
                outer = lambda r0, k0, nk: lin(SA[i], lambda r, k: w2t_v[r * DH + r0:r * DH + r0 + DQ, k * FH + k0:k * FH + k0 + nk].astype(f32))
                main = lin(SA[q], lambda r, k: outer(r * DQ, k * KS, KS))
                ar = lambda r: outer(r * DQ, 2 * KS, KT)
                extra = {2: lambda: ar(0), 5: lambda: ar(1) - ar(0), 3: lambda: ar(1), 6: lambda: ar(0) - ar(1)}.get(q)
                if extra is not None:
                    main = jnp.concatenate([main, extra()], axis=1)
                A22[(i, q)] = main.astype(bf)
            return A22[(i, q)]

        def mm2(s0, W2, nsteps, order=None, last=False):
            if s0 not in GEN:
                GEN[s0] = mm2gen(s0, W2, order, last)
            for _ in range(nsteps):
                next(GEN[s0])

        def mm2gen(s0, W2, order, last):
            w = W2 // 2; wq = w // 2
            P = [None] * 7
            def b2l2(i, q):
                outer = lambda k0, nk, c0: lin(SB[i], lambda k, c: hs_v[k * FH + k0:k * FH + k0 + nk, s0 + c * w + c0:s0 + c * w + c0 + wq])
                main = lin(SB[q], lambda k, c: outer(k * KS, KS, c * wq))
                cx = {2: 1, 5: 1, 3: 0, 6: 0}.get(q)
                if cx is not None:
                    main = jnp.concatenate([main, outer(2 * KS, KT, cx * wq)], axis=0)
                return main.astype(bf)
            for n, i in enumerate(order):
                P[i] = {}
                done_o = set(order[:n + 1])
                fin_o = [okey for okey, oterms in CN.items() if i in {t for _, t in oterms} and {t for _, t in oterms} <= done_o]
                split = last and n == 6
                def emit(key):
                    for okey in fin_o:
                        val = comb([None if p is None else p.get(key) for p in P], okey)
                        r0 = okey[0] * DH + key[0] * DQ; c0 = s0 + okey[1] * w + key[1] * wq
                        o_v[r0:r0 + DQ, c0:c0 + wq] = val.astype(bf)
                        if split:
                            out_copy(r0, DQ, c0, wq)
                if i not in l2set:
                    if i not in A21:
                        A21[i] = lin(SA[i], lambda r, k: w2t_v[r * DH:(r + 1) * DH, k * FH:(k + 1) * FH].astype(f32)).astype(bf)
                    gi = lin(SB[i], lambda k, c: hs_v[k * FH:(k + 1) * FH, s0 + c * w:s0 + (c + 1) * w]).astype(bf)
                    if not split:
                        full = dot(A21[i], gi)
                    for key in ((1, 0), (1, 1), (0, 1), (0, 0)):
                        rs = slice(key[0] * DQ, (key[0] + 1) * DQ); cs = slice(key[1] * wq, (key[1] + 1) * wq)
                        P[i][key] = dot(A21[i][rs], gi[:, cs]) if split else full[rs, cs]
                        emit(key)
                else:
                    ms = [None] * 7
                    for nq, q in enumerate(inner2):
                        ms[q] = dot(a2l2(i, q), b2l2(i, q))
                        done = set(inner2[:nq + 1])
                        for key, terms in CN.items():
                            need = {t for _, t in terms}
                            if q in need and need <= done:
                                P[i][key] = comb(ms, key)
                                emit(key)
                if last and not split:
                    for okey in fin_o:
                        out_copy(okey[0] * DH, DH, s0 + okey[1] * w, w)
                if not last and n == 6:
                    out_copy(0, D, s0, W2)
                yield

        fns = dict(px=px, pw1=pw1, mm1=mm1, mm2=mm2)
        for k in range(nst):
            with scope(f"wait{k}"):
                for c in in_copies(k):
                    c.wait()
                if k == nst - 1:
                    pin.wait()
            with scope(f"stage{k}"):
                for op in plan[k][1]:
                    fns[op[0]](*op[1:])
        assert sum(cover) == F * S
        with scope("waitout"):
            for cp in outs:
                cp.wait()

    def fn(x, w1, w2):
        B = x.shape[0]
        xt = x.reshape(S, D).T
        w2t = w2.T
        out = pl.pallas_call(kernel,
            in_specs=[pl.BlockSpec(memory_space=pl.ANY)]*3,
            out_specs=pl.BlockSpec(memory_space=pl.ANY),
            out_shape=jax.ShapeDtypeStruct((D, S), x.dtype),
            scratch_shapes=[pltpu.VMEM((D, S + xpad), bf), pltpu.VMEM((D, F), bf), pltpu.VMEM((D, F), bf), pltpu.VMEM((D, S), bf),
                            pltpu.VMEM((F, S + hpad), f32),
                            pltpu.SemaphoreType.DMA((nst,))],
            compiler_params=pltpu.CompilerParams(vmem_limit_bytes=120*1024*1024),
        )(xt, w1, w2t)
        return out.T.reshape(B, S, D)
    return fn

OF = (3, 5, 2, 0, 1, 6, 4); OM = (1, 5, 3, 0, 2, 6, 4); OL = (1, 5, 3, 0, 2, 4, 6)
def final_ops(chunks_old, fnew):
    big = sorted(chunks_old, key=lambda c: -c[1])
    ops = [('mm1', f0, nf, 1024, 512, 'nb' if n == 0 else 'std') for n, (f0, nf) in enumerate(big)]
    ops += [('mm1', f0, nf, 1024, 512, 'na') for (f0, nf) in fnew]
    ops += [('mm1', f0, nf, 0, 512) for (f0, nf) in fnew]
    for n in range(7):
        ops += [('mm2', 1024, 512, 1, OF), ('mm2', 0, 512, 1, OF)]
    ops += [('mm1', f0, nf, 512, 512) for (f0, nf) in fnew]
    ops += [('mm2', 512, 512, 7, OM)]
    allc = sorted(chunks_old + fnew, key=lambda c: -c[1])
    ops += [('mm1', f0, nf, 1536, 512) for (f0, nf) in allc]
    ops += [('mm2', 1536, 512, 7, OL, True)]
    return ops

def planA(v=0, **kw):
    if v == 0:
        plan = [([('w1', 0, 256)], [('pw1', 0, 256)]),
                ([('x', 0, 512)], [('mm1', 0, 256, 0, 512, 'nb')]),
                ([('w1', 256, 768)], [('mm1', 256, 512, 0, 512, 'na')]),
                ([('w1', 768, 1280), ('x', 512, 1024)], [('mm1', 256, 512, 512, 512, 'nb'), ('mm1', 0, 256, 512, 512), ('mm1', 768, 512, 0, 512, 'na'), ('mm1', 768, 512, 512, 512)]),
                ([('w1', 1280, 1792), ('x', 1024, 2048), ('w2', 0, 1792)], final_ops([(0, 256), (256, 512), (768, 512)], [(1280, 512)]))]
    if v == 1:
        plan = [([('w1', 0, 256)], [('pw1', 0, 256)]),
                ([('x', 0, 256)], [('mm1', 0, 256, 0, 256, 'nb')]),
                ([('x', 256, 512)], [('mm1', 0, 256, 256, 256, 'nb')]),
                ([('w1', 256, 768)], [('mm1', 256, 512, 0, 512, 'na')]),
                ([('w1', 768, 1280), ('x', 512, 1024)], [('mm1', 256, 512, 512, 512, 'nb'), ('mm1', 0, 256, 512, 512), ('mm1', 768, 512, 0, 512, 'na'), ('mm1', 768, 512, 512, 512)]),
                ([('w1', 1280, 1792), ('x', 1024, 2048), ('w2', 0, 1792)], final_ops([(0, 256), (256, 512), (768, 512)], [(1280, 512)]))]
    if v == 2:
        plan = [([('w1', 0, 256)], [('pw1', 0, 256)]),
                ([('x', 0, 256)], [('mm1', 0, 256, 0, 256, 'nb')]),
                ([('x', 256, 512), ('w1', 256, 512)], [('mm1', 0, 256, 256, 256, 'nb'), ('mm1', 256, 256, 0, 512, 'na')]),
                ([('w1', 512, 768), ('x', 512, 1024)], [('mm1', 0, 256, 512, 512, 'nb'), ('mm1', 256, 256, 512, 512), ('mm1', 512, 256, 0, 512, 'na'), ('mm1', 512, 256, 512, 512)]),
                ([('w1', 768, 1792), ('x', 1024, 1536)], [('mm1', 0, 256, 1024, 512, 'nb'), ('mm1', 256, 256, 1024, 512), ('mm1', 512, 256, 1024, 512),
                                                          ('mm1', 768, 512, 1024, 512, 'na'), ('mm1', 768, 512, 0, 512), ('mm1', 768, 512, 512, 512)]),
                ([('x', 1536, 2048), ('w2', 0, 1792)], [('mm1', 1280, 512, 1024, 512, 'na'), ('mm1', 1280, 512, 0, 512)] +
                    sum([[('mm2', 1024, 512, 1, OF), ('mm2', 0, 512, 1, OF)] for _ in range(7)], []) +
                    [('mm1', 1280, 512, 512, 512), ('mm2', 512, 512, 7, OM), ('mm1', 768, 512, 1536, 512), ('mm1', 1280, 512, 1536, 512), ('mm1', 0, 256, 1536, 512), ('mm1', 256, 256, 1536, 512), ('mm1', 512, 256, 1536, 512),
                     ('mm2', 1536, 512, 7, OL, True)])]
    return make(plan, **kw)


def planB(OF=OF, OM=OM, OL=OL, fv=0, pair=True, **kw):
    old = [(256, 512), (768, 512), (0, 256)]; new = (1280, 512)
    M1 = lambda c, t, o='std': ('mm1', c[0], c[1], 512 * t, 512, o)
    M2 = lambda t, n, o, last=False: ('mm2', 512 * t, 512, n, o, last)
    def pairs(a, b):
        if pair: return sum([[M2(a, 1, OF), M2(b, 1, OF)] for _ in range(7)], [])
        return [M2(a, 7, OF), M2(b, 7, OM)]
    t2old = [M1(old[0], 2, 'nb'), M1(old[1], 2), M1(old[2], 2)]
    t3all = [M1(old[0], 3), M1(old[2], 3), M1(old[1], 3), M1(new, 3)]
    if fv == 0:
        ops = t2old + [M1(new, 2, 'na'), M1(new, 0)] + pairs(2, 0) + [M1(new, 1), M2(1, 7, OM)] + t3all + [M2(3, 7, OL, True)]
    if fv == 1:
        ops = [M1(old[0], 2, 'nb'), M1(new, 0, 'na'), M1(new, 1), M1(old[1], 2)] + pairs(0, 1) + [M1(old[2], 2), M1(new, 2), M2(2, 7, OM)] + t3all + [M2(3, 7, OL, True)]
    if fv == 2:
        ops = t2old + [M1(new, 2, 'na'), M1(new, 0), M1(new, 1)] + pairs(2, 0) + [M2(1, 7, OM)] + t3all + [M2(3, 7, OL, True)]
    if fv == 3:
        ops = [M1(old[0], 2, 'nb'), M1(new, 0, 'na'), M1(new, 1), M1(old[1], 2)] + pairs(0, 1) + [M1(new, 2), M1(old[2], 2), M1(old[0], 3), M2(2, 7, OM)] + t3all[1:] + [M2(3, 7, OL, True)]
    plan = [([('w1', 0, 256)], [('pw1', 0, 256)]),
            ([('x', 0, 512)], [('mm1', 0, 256, 0, 512, 'nb')]),
            ([('w1', 256, 768)], [('mm1', 256, 512, 0, 512, 'na')]),
            ([('w1', 768, 1280), ('x', 512, 1024)], [('mm1', 256, 512, 512, 512, 'nb'), ('mm1', 0, 256, 512, 512), ('mm1', 768, 512, 0, 512, 'na'), ('mm1', 768, 512, 512, 512)]),
            ([('w1', 1280, 1792), ('x', 1024, 2048), ('w2', 0, 1792)], ops)]
    return make(plan, **kw)


def planC(v=0, OF=(5, 3, 2, 0, 1, 6, 4), OM=OM, OL=OL, **kw):
    M1 = lambda c, t, o='std': ('mm1', c[0], c[1], 512 * t, 512, o)
    M2 = lambda t, n, o, last=False: ('mm2', 512 * t, 512, n, o, last)
    pairs = lambda a, b: sum([[M2(a, 1, OF), M2(b, 1, OF)] for _ in range(7)], [])
    def fin(old, new):
        big = sorted(old, key=lambda c: -c[1])
        t2old = [M1(c, 2, 'nb' if n == 0 else 'std') for n, c in enumerate(big)]
        t3all = [M1(big[0], 3)] + [M1(c, 3) for c in sorted(big[1:])] + [M1(new, 3)]
        return t2old + [M1(new, 2, 'na'), M1(new, 0)] + pairs(2, 0) + [M1(new, 1), M2(1, 7, OM)] + t3all + [M2(3, 7, OL, True)]
    LF = [('w1', 1280, 1792), ('x', 1024, 2048), ('w2', 0, 1792)]
    a, b, c, d = (0, 256), (256, 512), (768, 512), (1280, 512)
    if v == 0:
        plan = [([('x', 0, 512)], [('px', 0, 512)]),
                ([('w1', 0, 256)], [M1(a, 0, 'na')]),
                ([('w1', 256, 768)], [M1(b, 0, 'na')]),
                ([('w1', 768, 1280), ('x', 512, 1024)], [M1(b, 1, 'nb'), M1(a, 1), M1(c, 0, 'na'), M1(c, 1)]),
                (LF, fin([a, b, c], d))]
    if v == 1:
        a2 = (0, 512); b2 = (512, 256)
        plan = [([('w1', 0, 512)], [('pw1', 0, 512)]),
                ([('x', 0, 256)], [('mm1', 0, 512, 0, 256, 'nb')]),
                ([('x', 256, 512), ('w1', 512, 768)], [('mm1', 0, 512, 256, 256, 'nb'), M1(b2, 0, 'na')]),
                ([('w1', 768, 1280), ('x', 512, 1024)], [M1(a2, 1, 'nb'), M1(b2, 1), M1(c, 0, 'na'), M1(c, 1)]),
                (LF, fin([a2, b2, c], d))]
    if v == 2:
        a1 = (0, 256); a2 = (256, 256); b2 = (512, 256)
        plan = [([('w1', 0, 256)], [('pw1', 0, 256)]),
                ([('w1', 256, 512)], [('pw1', 256, 256)]),
                ([('x', 0, 256)], [('mm1', 0, 256, 0, 256, 'nb'), ('mm1', 256, 256, 0, 256)]),
                ([('x', 256, 512), ('w1', 512, 768)], [('mm1', 0, 256, 256, 256, 'nb'), ('mm1', 256, 256, 256, 256), M1(b2, 0, 'na')]),
                ([('w1', 768, 1280), ('x', 512, 1024)], [M1(a1, 1, 'nb'), M1(a2, 1), M1(b2, 1), M1(c, 0, 'na'), M1(c, 1)]),
                (LF, fin([a1, a2, b2, c], d))]
    if v == 3:
        a1 = (0, 256); a2 = (256, 256); b2 = (512, 256)
        plan = [([('w1', 0, 256)], [('pw1', 0, 256)]),
                ([('x', 0, 256)], [('mm1', 0, 256, 0, 256, 'nb')]),
                ([('w1', 256, 512)], [('mm1', 256, 256, 0, 256, 'na')]),
                ([('x', 256, 512), ('w1', 512, 768)], [('mm1', 0, 256, 256, 256, 'nb'), ('mm1', 256, 256, 256, 256), M1(b2, 0, 'na')]),
                ([('w1', 768, 1280), ('x', 512, 1024)], [M1(a1, 1, 'nb'), M1(a2, 1), M1(b2, 1), M1(c, 0, 'na'), M1(c, 1)]),
                (LF, fin([a1, a2, b2, c], d))]
    return make(plan, **kw)


_impl = planB(OF=(5,3,2,4,6,0,1),OM=(5,4,1,6,3,2,0),OL=(1,3,2,0,4,5,6),fv=0,inner1=(2,4,3,0,6,1,5),inner2=(1,3,6,2,0,5,4),ords=dict(std=(0,3,4,2,6,1,5),nb=(1,4,3,0,6,2,5),na=(4,3,2,0,6,1,5)))


@jax.jit
def pallas_standalone__dense_activation_silu__prompt_kernel(x, w1, w2):
    return _impl(x, w1, w2)
```

```python
import jax
import jax.numpy as jnp
from jax.experimental import pallas as pl
from jax.experimental.pallas import tpu as pltpu

D, S, F = 448, 2048, 1792
KT = 128
FH = F // 2
DH = D // 2
DQ = D // 4
KS = 384
TS = 512
PAD = 128
bf = jnp.bfloat16
f32 = jnp.float32

SA = [((1, 0, 0), (1, 1, 1)), ((1, 1, 0), (1, 1, 1)), ((1, 0, 0),), ((1, 1, 1),),
      ((1, 0, 0), (1, 0, 1)), ((1, 1, 0), (-1, 0, 0)), ((1, 0, 1), (-1, 1, 1))]
SB = [((1, 0, 0), (1, 1, 1)), ((1, 0, 0),), ((1, 0, 1), (-1, 1, 1)), ((1, 1, 0), (-1, 0, 0)),
      ((1, 1, 1),), ((1, 0, 0), (1, 0, 1)), ((1, 1, 0), (1, 1, 1))]
CN = {(0, 0): ((1, 0), (1, 3), (-1, 4), (1, 6)), (0, 1): ((1, 2), (1, 4)),
      (1, 0): ((1, 1), (1, 3)), (1, 1): ((1, 0), (-1, 1), (1, 2), (1, 5))}
NESTED = (1, 2, 3, 4)

LOADS = [[('w1', 0, 256)],
         [('x', 0, 512)],
         [('w1', 256, 768)],
         [('w1', 768, 1280), ('x', 512, 1024)],
         [('w1', 1280, 1792), ('x', 1024, 2048), ('w2', 0, 1792)]]
CHUNK = dict(a=(0, 256), b=(256, 512), c=(768, 512), d=(1280, 512))
STAGES = [['W'], ['a0'], ['b0'], ['b1', 'a1', 'c0', 'c1'],
          ['b2', 'c2', 'a2', 'd2', 'd0',
           'P2', 'P0', 'P2', 'P0', 'P2', 'P0', 'P2', 'P0', 'P2', 'P2', 'P0', 'P2', 'P0', 'P0',
           'd1'] + ['P1'] * 7 + ['b3', 'a3', 'c3', 'd3'] + ['P3'] * 7]
LAST_TILE = 3
ORDER = {
    'a0': ((1, 4, 3, 0, 6, 2, 5), (2, 4, 3, 0, 6, 1, 5)), 'a1': ((0, 3, 4, 2, 6, 1, 5), (4, 2, 3, 0, 6, 1, 5)),
    'a2': ((0, 3, 4, 2, 6, 1, 5), (2, 4, 0, 3, 6, 1, 5)), 'a3': ((1, 4, 2, 0, 6, 3, 5), (2, 4, 3, 0, 6, 1, 5)),
    'b0': ((4, 3, 2, 0, 6, 1, 5), (2, 4, 3, 0, 6, 1, 5)), 'b1': ((1, 4, 3, 0, 6, 2, 5), (2, 4, 3, 0, 6, 1, 5)),
    'b2': ((1, 4, 3, 0, 6, 2, 5), (2, 4, 1, 0, 6, 3, 5)), 'b3': ((0, 3, 4, 6, 2, 1, 5), (2, 4, 3, 1, 0, 6, 5)),
    'c0': ((4, 3, 2, 0, 6, 1, 5), (2, 4, 3, 0, 6, 1, 5)), 'c1': ((0, 3, 4, 2, 6, 1, 5), (2, 4, 3, 0, 6, 1, 5)),
    'c2': ((0, 4, 2, 6, 3, 1, 5), (2, 4, 3, 0, 6, 1, 5)), 'c3': ((0, 6, 4, 2, 3, 1, 5), (2, 4, 3, 0, 6, 1, 5)),
    'd0': ((0, 4, 3, 2, 6, 1, 5), (2, 4, 3, 0, 1, 6, 5)), 'd1': ((0, 4, 6, 3, 2, 1, 5), (2, 3, 4, 0, 6, 1, 5)),
    'd2': ((4, 3, 2, 0, 6, 1, 5), (2, 4, 3, 0, 6, 1, 5)), 'd3': ((0, 3, 4, 2, 6, 1, 5), (2, 4, 3, 5, 6, 0, 1)),
    'P2': ((5, 3, 2, 4, 6, 0, 1), (1, 3, 0, 6, 2, 5, 4)), 'P0': ((5, 3, 2, 4, 6, 0, 1), (1, 3, 6, 2, 0, 5, 4)),
    'P1': ((5, 4, 1, 6, 3, 2, 0), (1, 6, 2, 3, 0, 5, 4)), 'P3': ((5, 3, 2, 4, 1, 0, 6), (1, 3, 6, 2, 0, 5, 4)),
}


def _dot(a, b):
    return jnp.dot(a, b, preferred_element_type=f32)


def _add(u, v):
    return (u.astype(f32) + v.astype(f32)).astype(bf)


def _sub(u, v):
    return (u.astype(f32) - v.astype(f32)).astype(bf)


def _up(u):
    return u.astype(f32)


def _silu(h):
    hh = 0.5 * h
    return hh + hh * jnp.tanh(hh)


def _lin(terms, get):
    acc = None
    for (c, u, v) in terms:
        t = get(u, v)
        acc = t if acc is None else (acc + t if c > 0 else acc - t)
    return acc


def _comb(ms, key):
    acc = None
    for (c, t) in CN[key]:
        acc = ms[t] if acc is None else (acc + ms[t] if c > 0 else acc - ms[t])
    return acc


def _rows(*u):
    return jnp.concatenate(u, axis=0)


def _kernel(xt_hbm, w1_hbm, w2t_hbm, o_hbm, xt_v, w1_v, w2t_v, o_v, h_v, sems):
    nst = len(STAGES)
    bufs = dict(x=(xt_hbm, xt_v), w1=(w1_hbm, w1_v), w2=(w2t_hbm, w2t_v))

    def in_copies(k):
        cps = []
        for (name, c0, c1) in LOADS[k]:
            src, dst = bufs[name]
            cps.append(pltpu.make_async_copy(src.at[:, pl.ds(c0, c1 - c0)],
                                             dst.at[:, pl.ds(c0, c1 - c0)], sems.at[k]))
        return cps

    outs = []

    def out_copy(r0, nr, c0, w):
        cp = pltpu.make_async_copy(o_v.at[pl.ds(r0, nr), pl.ds(c0, w)],
                                   o_hbm.at[pl.ds(r0, nr), pl.ds(c0, w)], sems.at[0])
        cp.start()
        outs.append(cp)

    pin = pltpu.make_async_copy(h_v.at[pl.ds(0, 8), pl.ds(S, PAD)],
                                h_v.at[pl.ds(8, 8), pl.ds(S, PAD)], sems.at[1])
    for k in range(nst):
        for c in in_copies(k):
            c.start()
        if k == 0:
            h_v[0:8, S:S + PAD] = jnp.zeros((8, PAD), f32)
            pin.start()

    lhs1, rhs1, lhs2_nested, lhs2_plain, mm2_state = {}, {}, {}, {}, {}

    def prep_w1(f0, nf):
        if (f0, nf) in lhs1:
            return lhs1[(f0, nf)]
        g = nf // 2
        tc = slice(f0, f0 + g)
        bc = slice(f0 + g, f0 + nf)
        top = w1_v[:2 * KT, tc].T
        bot = w1_v[:2 * KT, bc].T
        a11, a12 = top[:, :KT], top[:, KT:]
        a21, a22 = bot[:, :KT], bot[:, KT:]
        a1, a2, a3 = w1_v[256:320, tc], w1_v[320:384, tc], w1_v[384:448, tc]
        d1, d2, d3 = w1_v[256:320, bc], w1_v[320:384, bc], w1_v[384:448, bc]
        at = _rows(a1, _sub(a2, d2)).T
        ab = _rows(d1, _sub(d3, a3)).T
        az = _rows(d2, a3).T
        halves = [None, (lambda: _up(a21) + _up(a22), ab), (lambda: a11, az), (lambda: a22, az),
                  (lambda: _up(a11) + _up(a12), at), (lambda: _up(a21) - _up(a11), ab),
                  (lambda: _up(a12) - _up(a22), at)]
        res = [_add(a11, a22)]
        for i in range(1, 7):
            k0 = halves[i][0]()
            k1 = halves[i][1]
            if i in NESTED:
                gh = g // 2
                blk = lambda r, k: _up((k0, k1)[k][r * gh:(r + 1) * gh])
                res.append([_lin(SA[q], blk).astype(bf) for q in range(7)])
            else:
                res.append(jnp.concatenate([k0.astype(bf), k1], axis=1))
        lhs1[(f0, nf)] = res
        return res

    def prep_x(s0):
        if s0 in rhs1:
            return rhs1[s0]
        w = TS // 2
        L = slice(s0, s0 + w)
        R = slice(s0 + w, s0 + TS)
        b11, b12 = xt_v[:KT, L], xt_v[:KT, R]
        b21, b22 = xt_v[KT:2 * KT, L], xt_v[KT:2 * KT, R]
        lr = lambda r0, r1: _add(xt_v[r0:r1, L], xt_v[r0:r1, R])
        halves = [None,
                  (lambda: b11, lambda: _rows(xt_v[256:320, L], xt_v[384:448, L])),
                  (lambda: _up(b12) - _up(b22), lambda: xt_v[320:448, R]),
                  (lambda: _up(b21) - _up(b11), lambda: xt_v[320:448, L]),
                  (lambda: b22, lambda: xt_v[256:384, R]),
                  (lambda: lr(0, 128), lambda: _rows(lr(256, 320), lr(384, 448))),
                  (lambda: lr(128, 256), lambda: lr(256, 384))]
        res = [_add(b11, b22)]
        for i in range(1, 7):
            k0 = halves[i][0]()
            k1 = halves[i][1]()
            if i in NESTED:
                wh = w // 2
                blk = lambda k, c: _up((k0, k1)[k][:, c * wh:(c + 1) * wh])
                res.append([_lin(SB[q], blk).astype(bf) for q in range(7)])
            else:
                res.append(_rows(k0.astype(bf), k1))
        rhs1[s0] = res
        return res

    def mm1(f0, nf, s0, order, inner):
        A = prep_w1(f0, nf)
        B = prep_x(s0)
        g = nf // 2
        w = TS // 2
        m = [None] * 7
        for i in order:
            if i == 0:
                rs = g // 2
                m[i] = jnp.concatenate([_dot(A[i][r:r + rs], B[i]) for r in range(0, g, rs)], axis=0)
            elif i in NESTED:
                ms = [None] * 7
                for q in inner:
                    ms[q] = _dot(A[i][q], B[i][q])
                m[i] = jnp.concatenate(
                    [jnp.concatenate([_comb(ms, (r, c)) for c in range(2)], axis=1) for r in range(2)], axis=0)
            else:
                m[i] = _dot(A[i], B[i])
        m1, m2, m3, m4, m5, m6, m7 = m
        h_v[f0:f0 + g, s0:s0 + w] = _silu(m1 + m4 - m5 + m7)
        h_v[f0:f0 + g, s0 + w:s0 + TS] = _silu(m3 + m5)
        h_v[f0 + g:f0 + nf, s0:s0 + w] = _silu(m2 + m4)
        h_v[f0 + g:f0 + nf, s0 + w:s0 + TS] = _silu(m1 - m2 + m3 + m6)

    def w2_nested(i, q):
        if (i, q) not in lhs2_nested:
            outer = lambda r0, k0, nk: _lin(SA[i], lambda r, k: w2t_v[
                r * DH + r0:r * DH + r0 + DQ, k * FH + k0:k * FH + k0 + nk].astype(f32))
            main = _lin(SA[q], lambda r, k: outer(r * DQ, k * KS, KS))
            tail = lambda r: outer(r * DQ, 2 * KS, KT)
            extra = {2: lambda: tail(0), 5: lambda: tail(1) - tail(0),
                     3: lambda: tail(1), 6: lambda: tail(0) - tail(1)}.get(q)
            if extra is not None:
                main = jnp.concatenate([main, extra()], axis=1)
            lhs2_nested[(i, q)] = main.astype(bf)
        return lhs2_nested[(i, q)]

    def mm2_steps(s0, order, inner, last):
        w = TS // 2
        wq = w // 2
        P = [None] * 7

        def h_nested(i, q):
            outer = lambda k0, nk, c0: _lin(SB[i], lambda k, c: h_v[
                k * FH + k0:k * FH + k0 + nk, s0 + c * w + c0:s0 + c * w + c0 + wq])
            main = _lin(SB[q], lambda k, c: outer(k * KS, KS, c * wq))
            cx = {2: 1, 5: 1, 3: 0, 6: 0}.get(q)
            if cx is not None:
                main = jnp.concatenate([main, outer(2 * KS, KT, cx * wq)], axis=0)
            return main.astype(bf)

        for n, i in enumerate(order):
            P[i] = {}
            done_o = set(order[:n + 1])
            fin_o = [okey for okey, ot in CN.items()
                     if i in {t for _, t in ot} and {t for _, t in ot} <= done_o]
            split = last and n == 6

            def emit(key):
                for okey in fin_o:
                    val = _comb([None if p is None else p.get(key) for p in P], okey)
                    r0 = okey[0] * DH + key[0] * DQ
                    c0 = s0 + okey[1] * w + key[1] * wq
                    o_v[r0:r0 + DQ, c0:c0 + wq] = val.astype(bf)
                    if split:
                        out_copy(r0, DQ, c0, wq)

            if i not in NESTED:
                if i not in lhs2_plain:
                    lhs2_plain[i] = _lin(SA[i], lambda r, k: w2t_v[
                        r * DH:(r + 1) * DH, k * FH:(k + 1) * FH].astype(f32)).astype(bf)
                gi = _lin(SB[i], lambda k, c: h_v[
                    k * FH:(k + 1) * FH, s0 + c * w:s0 + (c + 1) * w]).astype(bf)
                if not split:
                    full = _dot(lhs2_plain[i], gi)
                for key in ((1, 0), (1, 1), (0, 1), (0, 0)):
                    rs = slice(key[0] * DQ, (key[0] + 1) * DQ)
                    cs = slice(key[1] * wq, (key[1] + 1) * wq)
                    P[i][key] = _dot(lhs2_plain[i][rs], gi[:, cs]) if split else full[rs, cs]
                    emit(key)
            else:
                ms = [None] * 7
                for nq, q in enumerate(inner):
                    ms[q] = _dot(w2_nested(i, q), h_nested(i, q))
                    done = set(inner[:nq + 1])
                    for key, terms in CN.items():
                        need = {t for _, t in terms}
                        if q in need and need <= done:
                            P[i][key] = _comb(ms, key)
                            emit(key)
            if last and not split:
                for okey in fin_o:
                    out_copy(okey[0] * DH, DH, s0 + okey[1] * w, w)
            if not last and n == 6:
                out_copy(0, D, s0, TS)
            yield

    for k in range(nst):
        for c in in_copies(k):
            c.wait()
        if k == 1:
            pin.wait()
        for tok in STAGES[k]:
            if tok == 'W':
                prep_w1(*CHUNK['a'])
            elif tok[0] == 'P':
                t = int(tok[1])
                if t not in mm2_state:
                    mm2_state[t] = mm2_steps(TS * t, *ORDER[tok], t == LAST_TILE)
                next(mm2_state[t])
            else:
                mm1(*CHUNK[tok[0]], TS * int(tok[1]), *ORDER[tok])
    for cp in outs:
        cp.wait()


@jax.jit
def pallas_standalone__dense_activation_silu__prompt_kernel(
    x: jax.Array,
    w1: jax.Array,
    w2: jax.Array,
):
    B = x.shape[0]
    assert x.shape == (1, S, D) and w1.shape == (D, F) and w2.shape == (F, D)
    xt = x.reshape(S, D).T
    w2t = w2.T
    out_t = pl.pallas_call(
        _kernel,
        in_specs=[pl.BlockSpec(memory_space=pl.ANY)] * 3,
        out_specs=pl.BlockSpec(memory_space=pl.ANY),
        out_shape=jax.ShapeDtypeStruct((D, S), x.dtype),
        scratch_shapes=[
            pltpu.VMEM((D, S + PAD), bf),
            pltpu.VMEM((D, F), bf),
            pltpu.VMEM((D, F), bf),
            pltpu.VMEM((D, S), bf),
            pltpu.VMEM((F, S + PAD), f32),
            pltpu.SemaphoreType.DMA((len(STAGES),)),
        ],
        compiler_params=pltpu.CompilerParams(vmem_limit_bytes=64 * 1024 * 1024),
    )(xt, w1, w2t)
    return out_t.T.reshape(B, S, D)
```
